```python
import os as _os
_os.environ.setdefault("JAX_PLATFORMS", "cpu")
import jax
import jax.numpy as jnp

def _softmax(x, axis=-1):
    return jax.nn.softmax(x, axis=axis)
def _gelu(x):
    return jax.nn.gelu(x, approximate=True)
def _silu(x):
    return jax.nn.silu(x)
def _sigmoid(x):
    return jax.nn.sigmoid(x)
def _layernorm(x, axis=-1, eps=1e-5):
    m = jnp.mean(x, axis=axis, keepdims=True)
    v = jnp.var(x, axis=axis, keepdims=True)
    return (x - m) / jnp.sqrt(v + eps)
def _scatter_add(tgt, idx, src, axis=0):
    return tgt.at[idx].add(src)
def _segment_sum(src, seg, n):
    return jax.ops.segment_sum(src, seg, n)
class _Rng:
    def __init__(self, key):
        self._k = key
    def _next(self):
        self._k, sub = jax.random.split(self._k)
        return sub
    def normal(self, shape):
        return jax.random.normal(self._next(), shape, dtype=jnp.bfloat16)
    def randint(self, lo, hi, shape):
        return jax.random.randint(self._next(), shape, lo, hi, dtype=jnp.int32)
    def uniform(self, shape, lo=0.0, hi=1.0):
        return jax.random.uniform(self._next(), shape, jnp.bfloat16, lo, hi)
    def permutation(self, n):
        return jax.random.permutation(self._next(), n)


kernel_name = 'gated_mix__ssm_conv_s5__glu_gated_geglu__prompt'

def setup_inputs():
    _rng = _Rng(jax.random.key(int.from_bytes(__import__("os").urandom(4), "little")))
    _w = (lambda a: (lambda t: t.astype(jnp.bfloat16) if jnp.issubdtype(t.dtype, jnp.floating) else t)(jnp.asarray(a)))
    def _A_setup():
        B, S, D = 1, 2048, 448
        P = D
        Lambda_re = -0.5 * jnp.exp((lambda *s: _rng.normal(s) * 0.4)(P))
        Lambda_im = (lambda *s: _rng.normal(s) * 0.4)(P) * 1.0
        B_re = (lambda *s: _rng.normal(s) * 0.4)(P, D) * (D ** -0.5)
        B_im = (lambda *s: _rng.normal(s) * 0.4)(P, D) * (D ** -0.5)
        C_re = (lambda *s: _rng.normal(s) * 0.4)(D, P) * (P ** -0.5)
        C_im = (lambda *s: _rng.normal(s) * 0.4)(D, P) * (P ** -0.5)
        log_dt = (lambda *s: _rng.normal(s) * 0.4)(P) * 0.3 - 2.0
        Dskip = (lambda *s: _rng.normal(s) * 0.4)(D)
        return {
            "x": _w((lambda *s: _rng.normal(s) * 0.05)(B, S, D)),
            "Lambda_re": _w(Lambda_re),
            "Lambda_im": _w(Lambda_im),
            "B_re": _w(B_re),
            "B_im": _w(B_im),
            "C_re": _w(C_re),
            "C_im": _w(C_im),
            "log_dt": _w(log_dt),
            "Dskip": _w(Dskip),
        }
    _A_in = _A_setup()

    def _B_setup():
        B, S, Dm, Df = 1, 2048, 448, 1792
        return {
            "x": _w((lambda *s: _rng.normal(s) * 0.05)(B, S, Dm)),
            "w_gate": _w((lambda *s: _rng.normal(s) * 1.6)(Dm, Df) * (Dm ** -0.5)),
            "w_up": _w((lambda *s: _rng.normal(s) * 1.6)(Dm, Df) * (Dm ** -0.5)),
            "w_down": _w((lambda *s: _rng.normal(s) * 1.6)(Df, Dm) * (Df ** -0.5)),
        }
    _B_in = _B_setup()

    return {
        "A_x": _A_in["x"],
        "A_Lambda_re": _A_in["Lambda_re"],
        "A_Lambda_im": _A_in["Lambda_im"],
        "A_B_re": _A_in["B_re"],
        "A_B_im": _A_in["B_im"],
        "A_C_re": _A_in["C_re"],
        "A_C_im": _A_in["C_im"],
        "A_log_dt": _A_in["log_dt"],
        "A_Dskip": _A_in["Dskip"],
        "B_x": _B_in["x"],
        "B_w_gate": _B_in["w_gate"],
        "B_w_up": _B_in["w_up"],
        "B_w_down": _B_in["w_down"],
        "gate_w": _w((lambda *s: _rng.normal(s) * 0.05)(448) * 16.0),
    }

def reference(A_x, A_Lambda_re, A_Lambda_im, A_B_re, A_B_im, A_C_re, A_C_im, A_log_dt, A_Dskip, B_x, B_w_gate, B_w_up, B_w_down, gate_w):
    def _A_ref(x, Lambda_re, Lambda_im, B_re, B_im, C_re, C_im, log_dt, Dskip):
        Bsz, L, H = x.shape
        Lam = Lambda_re + 1j * Lambda_im
        Bmat = B_re + 1j * B_im
        Cmat = C_re + 1j * C_im
        dt = jnp.exp(log_dt)
        Lam_bar = jnp.exp(dt * Lam)
        B_bar = ((Lam_bar - 1.0) / Lam)[:, None] * Bmat
        Bu = jnp.einsum("bld,pd->blp", x + 0j, B_bar)
        h = jnp.zeros_like(Bu[:, 0, :])
        hs = []
        for t in range(L):
            h = Lam_bar[None, :] * h + Bu[:, t, :]
            hs.append(h)
        hseq = jnp.stack(hs, 1)
        y = 2.0 * jnp.einsum("blp,dp->bld", hseq, Cmat).real + x * Dskip[None, None, :]
        return y

    def _B_ref(x, w_gate, w_up, w_down):
        g = jnp.einsum("bsd,df->bsf", x, w_gate)
        u = jnp.einsum("bsd,df->bsf", x, w_up)
        h = _gelu(g) * u
        return jnp.einsum("bsf,fd->bsd", h, w_down)

    x = A_x
    g = _sigmoid((x * gate_w).sum(-1, keepdims=True))
    a = _A_ref(x, A_Lambda_re, A_Lambda_im, A_B_re, A_B_im, A_C_re, A_C_im, A_log_dt, A_Dskip)
    b = _B_ref(x, B_w_gate, B_w_up, B_w_down)
    return g * a + (1 - g) * b
```

```python
import functools
import numpy as np
import jax
import jax.numpy as jnp
import jax.experimental.pallas as pl
import jax.experimental.pallas.tpu as pltpu

CFG = dict(M=512, FB=256)
def configure(**kw):
    CFG.update(kw)

F32 = jnp.float32
BF16 = jnp.bfloat16


def _nt(a, b):
    return jax.lax.dot_general(a, b, (((1,), (1,)), ((), ())), preferred_element_type=F32)


def _kernel(xt_ref, lre_ref, lim_ref, bre_ref, bim_ref, cre_ref, cim_ref, ldt_ref, dsk_ref,
            wg_ref, wu_ref, wdt_ref, gw_ref, o_ref,
            cre_s, cim_s, const_s, hc_s, col_s, *, M, FB):
    step = pl.program_id(0)

    @pl.when(step == 0)
    def _prep():
        lre = lre_ref[...].astype(F32).reshape(1, 448)
        lim = lim_ref[...].astype(F32).reshape(1, 448)
        dt = jnp.exp(ldt_ref[...].astype(F32).reshape(1, 448)).astype(BF16).astype(F32)
        ar = dt * lre
        ai = dt * lim
        k = (jax.lax.broadcasted_iota(jnp.int32, (8, 448), 0) + 1).astype(F32)
        mag = jnp.exp(k * ar)
        pr = mag * jnp.cos(k * ai)
        pi_ = mag * jnp.sin(k * ai)
        row = jax.lax.broadcasted_iota(jnp.int32, (8, 448), 0)
        const_s[0] = pr
        const_s[1] = pi_
        for n, kk in enumerate((1, 2, 4)):
            const_s[2 + 2 * n] = jnp.where(row >= kk, pr[kk - 1:kk, :], 0.0)
            const_s[3 + 2 * n] = jnp.where(row >= kk, pi_[kk - 1:kk, :], 0.0)
        nr = pr[0:1, :] - 1.0
        ni = pi_[0:1, :]
        den = 1.0 / (lre * lre + lim * lim)
        cr = (nr * lre + ni * lim) * den
        ci = (ni * lre - nr * lim) * den
        c_re = cre_ref[...].astype(F32)
        c_im = cim_ref[...].astype(F32)
        cre_s[...] = (2.0 * (c_re * cr - c_im * ci)).astype(BF16)
        cim_s[...] = (-2.0 * (c_re * ci + c_im * cr)).astype(BF16)
        hc_s[...] = jnp.zeros_like(hc_s)
        gw8 = jnp.broadcast_to(gw_ref[...].astype(F32).reshape(1, 448), (128, 448))
        ds8 = jnp.broadcast_to(dsk_ref[...].astype(F32).reshape(1, 448), (128, 448))
        col_s[0] = gw8.T
        col_s[1] = ds8.T

    xt = xt_ref[...]
    x = xt.T
    xtf = xt.astype(F32)
    vre = _nt(x, bre_ref[...]).reshape(M // 8, 8, 448)
    vim = _nt(x, bim_ref[...]).reshape(M // 8, 8, 448)
    for n, kk in enumerate((1, 2, 4)):
        a_re = const_s[2 + 2 * n][None]
        a_im = const_s[3 + 2 * n][None]
        s_re = pltpu.roll(vre, kk, 1)
        s_im = pltpu.roll(vim, kk, 1)
        vre, vim = vre + (a_re * s_re - a_im * s_im), vim + (a_re * s_im + a_im * s_re)
    p_re = const_s[0]
    p_im = const_s[1]
    c_re = hc_s[0]
    c_im = hc_s[1]
    hre = []
    him = []
    for j in range(M // 8):
        b_re = jnp.broadcast_to(c_re[7:8, :], (8, 448))
        b_im = jnp.broadcast_to(c_im[7:8, :], (8, 448))
        c_re = vre[j] + (p_re * b_re - p_im * b_im)
        c_im = vim[j] + (p_re * b_im + p_im * b_re)
        hre.append(c_re)
        him.append(c_im)
    hc_s[0] = c_re
    hc_s[1] = c_im
    h_re = jnp.concatenate(hre, axis=0).astype(BF16)
    h_im = jnp.concatenate(him, axis=0).astype(BF16)
    acc = None
    for j in range(1792 // FB):
        g = jnp.dot(x, wg_ref[:, j * FB:(j + 1) * FB], preferred_element_type=F32)
        u = jnp.dot(x, wu_ref[:, j * FB:(j + 1) * FB], preferred_element_type=F32)
        inner = g * (0.7978845608028654 + (0.7978845608028654 * 0.044715) * (g * g))
        r = (0.5 * g) * u
        hh = (r + r * jnp.tanh(inner)).astype(BF16)
        d = _nt(wdt_ref[:, j * FB:(j + 1) * FB], hh)
        acc = d if acc is None else acc + d
    nrep = M // 128
    gwc = jnp.tile(col_s[0], (1, nrep))
    dsc = jnp.tile(col_s[1], (1, nrep))
    a = _nt(cre_s[...], h_re) + _nt(cim_s[...], h_im) + xtf * dsc
    logit = jnp.sum(xtf * gwc, axis=0, keepdims=True)
    gate = jax.nn.sigmoid(logit)
    o_ref[...] = acc + gate * (a - acc)


@jax.jit
def pallas_gated_mix__ssm_conv_s5__glu_gated_geglu__prompt_kernel(
    A_x, A_Lambda_re, A_Lambda_im, A_B_re, A_B_im, A_C_re, A_C_im, A_log_dt, A_Dskip,
    B_x, B_w_gate, B_w_up, B_w_down, gate_w,
):
    M = CFG["M"]
    _, S, D = A_x.shape
    F = B_w_gate.shape[1]
    vec = pl.BlockSpec((D,), lambda i: (0,))
    full = lambda a, b: pl.BlockSpec((a, b), lambda i: (0, 0))
    xt = jnp.transpose(A_x.reshape(S, D))
    wdt = jnp.transpose(B_w_down)
    out_t = pl.pallas_call(
        functools.partial(_kernel, M=M, FB=CFG["FB"]),
        grid=(S // M,),
        in_specs=[pl.BlockSpec((D, M), lambda i: (0, i)), vec, vec,
                  full(D, D), full(D, D), full(D, D), full(D, D), vec, vec,
                  full(D, F), full(D, F), full(D, F), vec],
        out_specs=pl.BlockSpec((D, M), lambda i: (0, i)),
        out_shape=jax.ShapeDtypeStruct((D, S), F32),
        scratch_shapes=[pltpu.VMEM((D, D), BF16), pltpu.VMEM((D, D), BF16),
                        pltpu.VMEM((8, 8, D), F32), pltpu.VMEM((2, 8, D), F32),
                        pltpu.VMEM((2, D, 128), F32)],
        compiler_params=pltpu.CompilerParams(dimension_semantics=("arbitrary",),
                                             vmem_limit_bytes=100 * 1024 * 1024),
    )(xt, A_Lambda_re, A_Lambda_im, A_B_re, A_B_im, A_C_re, A_C_im, A_log_dt, A_Dskip,
      B_w_gate, B_w_up, wdt, gate_w)
    return jnp.transpose(out_t).reshape(1, S, D)
```

```python
import functools
import numpy as np
import jax
import jax.numpy as jnp
import jax.experimental.pallas as pl
import jax.experimental.pallas.tpu as pltpu

CFG = dict(M=512, FT=128, RB=32, G2=6, B4=11, OSPLIT=4, fence=True)
def configure(**kw):
    CFG.update(kw)

F32 = jnp.float32
BF16 = jnp.bfloat16
D = 448
P2 = 896
F = 1792
S = 2048
C1 = 0.7978845608028654
C2 = 0.7978845608028654 * 0.044715


def _nt(a, b):
    return jax.lax.dot_general(a, b, (((1,), (1,)), ((), ())), preferred_element_type=F32)


def _kernel(xt_hbm, lre_hbm, lim_hbm, bre_hbm, bim_hbm, cre_hbm, cim_hbm, ldt_hbm, dsk_hbm,
            wg_hbm, wu_hbm, wdt_hbm, gw_hbm, o_hbm,
            xt_s, v0_s, v1_s, v2_s, v3_s, v4_s, bcat_s, wg_s, wu_s, wd_s, cre_s, cim_s, cp_s,
            const_s, hc_s, col_s, coef_s, o_s, sems, *, M, FT, RB, G2, B4, OSPLIT, fence):
    NC = S // M
    NT = F // FT
    NS = M // 128
    NG = M // 8
    vecs = (v0_s, v1_s, v2_s, v3_s, v4_s)

    def cp(src, dst, k):
        return pltpu.make_async_copy(src, dst, sems.at[k])

    fa = G2 * FT
    g_vec = [cp(src, vecs[n], 0) for n, src in enumerate((lre_hbm, lim_hbm, ldt_hbm, dsk_hbm, gw_hbm))]
    g_x0 = [cp(xt_hbm.at[:, pl.ds(0, M)], xt_s.at[0], 1)]
    g_b0 = [cp(bre_hbm.at[pl.ds(0, 384), :], bcat_s.at[pl.ds(0, 384), :], 2)]
    g_b1 = [cp(bim_hbm.at[pl.ds(0, 384), :], bcat_s.at[pl.ds(384, 384), :], 3),
            cp(bre_hbm.at[pl.ds(384, 64), :], bcat_s.at[pl.ds(768, 64), :], 3),
            cp(bim_hbm.at[pl.ds(384, 64), :], bcat_s.at[pl.ds(832, 64), :], 3)]
    g_w0 = [cp(wg_hbm.at[:, pl.ds(0, fa)], wg_s.at[:, pl.ds(0, fa)], 4),
            cp(wu_hbm.at[:, pl.ds(0, fa)], wu_s.at[:, pl.ds(0, fa)], 4)]
    g_w1 = [cp(wg_hbm.at[:, pl.ds(fa, F - fa)], wg_s.at[:, pl.ds(fa, F - fa)], 5),
            cp(wu_hbm.at[:, pl.ds(fa, F - fa)], wu_s.at[:, pl.ds(fa, F - fa)], 5)]
    g_w2 = [cp(wdt_hbm, wd_s, 6), cp(cre_hbm, cre_s, 6), cp(cim_hbm, cim_s, 6)]
    g_w2 += [cp(xt_hbm.at[:, pl.ds(i * M, M)], xt_s.at[i], 6) for i in range(1, NC)]

    def wait_all(group):
        for c in group:
            c.wait()

    def o_copy(i, s, r0, nr):
        return cp(o_s.at[i, pl.ds(r0, nr), pl.ds(s * 128, 128)],
                  o_hbm.at[pl.ds(r0, nr), pl.ds(i * M + s * 128, 128)], 7)

    for grp in (g_vec, g_x0, g_b0, g_b1, g_w0, g_w1, g_w2):
        for c in grp:
            c.start()

    wait_all(g_vec)

    def ext(v):
        return jnp.concatenate([v, v[:, 384:448]], axis=1)

    lre = vecs[0][...].astype(F32).reshape(1, D)
    lim = vecs[1][...].astype(F32).reshape(1, D)
    dt = jnp.exp(vecs[2][...].astype(F32).reshape(1, D)).astype(BF16).astype(F32)
    ar = dt * lre
    ai = dt * lim
    k8 = (jax.lax.broadcasted_iota(jnp.int32, (8, 512), 0) + 1).astype(F32)
    lane = jax.lax.broadcasted_iota(jnp.int32, (8, 512), 1)
    row = jax.lax.broadcasted_iota(jnp.int32, (8, 512), 0)
    sgn = jnp.where(lane >= 448, -1.0, 1.0)
    mag = jnp.exp(k8 * ext(ar))
    ang = k8 * ext(ai)
    pr = mag * jnp.cos(ang)
    pi_ = mag * jnp.sin(ang) * sgn
    const_s[0] = pr
    const_s[1] = pi_
    for n, kk in enumerate((1, 2, 4)):
        const_s[2 + 2 * n] = jnp.where(row >= kk, pr[kk - 1:kk, :], 0.0)
        const_s[3 + 2 * n] = jnp.where(row >= kk, pi_[kk - 1:kk, :], 0.0)
    hc_s[...] = jnp.zeros_like(hc_s)
    gw8 = jnp.broadcast_to(vecs[4][...].astype(F32).reshape(1, D), (128, D))
    ds8 = jnp.broadcast_to(vecs[3][...].astype(F32).reshape(1, D), (128, D))
    col_s[0] = gw8.T
    col_s[1] = ds8.T
    nr_ = pr[0:1, :D] - 1.0
    ni_ = pi_[0:1, :D]
    den = 1.0 / (lre * lre + lim * lim)
    coef_s[0] = jnp.broadcast_to(2.0 * ((nr_ * lre + ni_ * lim) * den), (8, D))
    coef_s[1] = jnp.broadcast_to(2.0 * ((ni_ * lre - nr_ * lim) * den), (8, D))

    def prep_c_block(r, cr8, ci8):
        rs = slice(r * 16, (r + 1) * 16)
        cr = jnp.concatenate([cr8, cr8], axis=0)
        ci = jnp.concatenate([ci8, ci8], axis=0)
        c_re = cre_s[rs, :].astype(F32)
        c_im = cim_s[rs, :].astype(F32)
        q_re = c_re * cr - c_im * ci
        q_im = -(c_re * ci + c_im * cr)
        cp_s[rs, 0:384] = q_re[:, 0:384].astype(BF16)
        cp_s[rs, 384:768] = q_im[:, 0:384].astype(BF16)
        cp_s[rs, 768:896] = jnp.concatenate([q_re[:, 384:448], q_im[:, 384:448]], axis=1).astype(BF16)

    def zero_after(piece):
        zz = jnp.where(piece[0:8, :] < -jnp.inf, 1.0, 0.0)
        return jnp.concatenate([zz] * 4, axis=1)

    def chunk(i, first):
        if first:
            wait_all(g_x0)
        xt = xt_s[i]
        x = xt.T
        if first:
            wait_all(g_b0)
        v_re = _nt(x, bcat_s[0:384, :])
        if first:
            wait_all(g_b1)
        v_im = _nt(x, bcat_s[384:768, :])
        v_t = _nt(x, bcat_s[768:896, :])
        if first:
            wait_all(g_w0)

        st = dict(c_re=hc_s[0], c_im=hc_s[1], g=0)
        hre = []
        him = []

        def scan_group(z):
            gidx = st["g"]
            cs = [const_s[q] for q in range(8)]
            if z is not None:
                cs[2] = cs[2] + z
                cs[3] = cs[3] + z
            rs = slice(gidx * 8, gidx * 8 + 8)
            t = v_t[rs, :]
            vre = jnp.concatenate([v_re[rs, :], t], axis=1)
            vim = jnp.concatenate([v_im[rs, :], pltpu.roll(t, 64, 1)], axis=1)
            for n_, kk in enumerate((1, 2, 4)):
                a_re = cs[2 + 2 * n_]
                a_im = cs[3 + 2 * n_]
                s_re = pltpu.roll(vre, kk, 0)
                s_im = pltpu.roll(vim, kk, 0)
                vre, vim = vre + (a_re * s_re - a_im * s_im), vim + (a_re * s_im + a_im * s_re)
            p_re = cs[0]
            p_im = cs[1]
            b_re = jnp.broadcast_to(st["c_re"][7:8, :], (8, 512))
            b_im = jnp.broadcast_to(st["c_im"][7:8, :], (8, 512))
            st["c_re"] = vre + (p_re * b_re - p_im * b_im)
            st["c_im"] = vim + (p_re * b_im + p_im * b_re)
            hre.append(st["c_re"])
            him.append(st["c_im"])
            st["g"] = gidx + 1

        hhs = []
        per = -(-NG // NT)
        cblk = 0
        npc = M // RB
        for j in range(NT):
            if first and j == G2:
                wait_all(g_w1)
            if first and j == B4:
                wait_all(g_w2)
            g = jnp.dot(x, wg_s[:, j * FT:(j + 1) * FT], preferred_element_type=F32)
            u = jnp.dot(x, wu_s[:, j * FT:(j + 1) * FT], preferred_element_type=F32)
            ng_here = min(per, NG - st["g"])
            g_trig = [(q * npc) // ng_here for q in range(ng_here)]
            c_trig = []
            if first and j >= B4:
                nblk = -(-(28 - cblk) // (NT - j))
                c_trig = [((2 * q + 1) * npc) // (2 * nblk) for q in range(nblk)]
            pieces = []
            for rb in range(npc):
                rs = slice(rb * RB, (rb + 1) * RB)
                gg = g[rs, :]
                inner = gg * (C1 + C2 * (gg * gg))
                r = (0.5 * gg) * u[rs, :]
                pieces.append(r + r * jnp.tanh(inner))
                z = None
                if fence and (rb in g_trig or rb in c_trig):
                    z = zero_after(pieces[-1])
                for _ in range(g_trig.count(rb)):
                    scan_group(z)
                for _ in range(c_trig.count(rb)):
                    cr8, ci8 = coef_s[0], coef_s[1]
                    if z is not None:
                        cr8, ci8 = cr8 + z[:, :D], ci8 + z[:, :D]
                    prep_c_block(cblk, cr8, ci8)
                    cblk += 1
            hhs.append(jnp.concatenate(pieces, axis=0))
        assert st["g"] == NG and (cblk == 28 or not first)
        hc_s[0] = st["c_re"]
        hc_s[1] = st["c_im"]
        h_re = jnp.concatenate(hre, axis=0)
        h_im = jnp.concatenate(him, axis=0)
        hp = jnp.concatenate([h_re[:, :384], h_im[:, :384], h_re[:, 384:]], axis=1)
        hh = jnp.concatenate(hhs, axis=1)
        for s in range(NS):
            sl = slice(s * 128, (s + 1) * 128)
            xtf = xt[:, sl].astype(F32)
            a = _nt(cp_s[...], hp[sl, :].astype(BF16)) + xtf * col_s[1]
            b = _nt(wd_s[...], hh[sl, :].astype(BF16))
            gate = jax.nn.sigmoid(jnp.sum(xtf * col_s[0], axis=0, keepdims=True))
            nsp = OSPLIT if s == NS - 1 else 1
            nr = D // nsp
            for q in range(nsp):
                rr = slice(q * nr, (q + 1) * nr)
                o_s[i, rr, sl] = b[rr, :] + gate * (a[rr, :] - b[rr, :])
                o_copy(i, s, q * nr, nr).start()

    chunk(0, True)

    def body(i, carry):
        chunk(i, False)
        return carry
    jax.lax.fori_loop(1, NC, body, 0)
    pltpu.make_async_copy(o_s, o_s, sems.at[7]).wait()


@jax.jit
def pallas_gated_mix__ssm_conv_s5__glu_gated_geglu__prompt_kernel(
    A_x, A_Lambda_re, A_Lambda_im, A_B_re, A_B_im, A_C_re, A_C_im, A_log_dt, A_Dskip,
    B_x, B_w_gate, B_w_up, B_w_down, gate_w,
):
    M = CFG["M"]
    NC = S // M
    xt = jnp.transpose(A_x.reshape(S, D))
    wdt = jnp.transpose(B_w_down)
    hbm = pl.BlockSpec(memory_space=pl.ANY)
    kw = {k: CFG[k] for k in ("M", "FT", "RB", "G2", "B4", "OSPLIT", "fence")}
    out_t = pl.pallas_call(
        functools.partial(_kernel, **kw),
        in_specs=[hbm] * 13,
        out_specs=hbm,
        out_shape=jax.ShapeDtypeStruct((D, S), F32),
        scratch_shapes=[
            pltpu.VMEM((NC, D, M), BF16),
            pltpu.VMEM((D,), BF16), pltpu.VMEM((D,), BF16), pltpu.VMEM((D,), BF16),
            pltpu.VMEM((D,), BF16), pltpu.VMEM((D,), BF16),
            pltpu.VMEM((P2, D), BF16),
            pltpu.VMEM((D, F), BF16),
            pltpu.VMEM((D, F), BF16),
            pltpu.VMEM((D, F), BF16),
            pltpu.VMEM((D, D), BF16),
            pltpu.VMEM((D, D), BF16),
            pltpu.VMEM((D, P2), BF16),
            pltpu.VMEM((8, 8, 512), F32),
            pltpu.VMEM((2, 8, 512), F32),
            pltpu.VMEM((2, D, 128), F32),
            pltpu.VMEM((2, 8, D), F32),
            pltpu.VMEM((NC, D, M), F32),
            pltpu.SemaphoreType.DMA((8,)),
        ],
        compiler_params=pltpu.CompilerParams(vmem_limit_bytes=100 * 1024 * 1024),
    )(xt, A_Lambda_re, A_Lambda_im, A_B_re, A_B_im, A_C_re, A_C_im, A_log_dt, A_Dskip,
      B_w_gate, B_w_up, wdt, gate_w)
    return jnp.transpose(out_t).reshape(1, S, D)
```

```python
import functools

import jax
import jax.numpy as jnp
import jax.experimental.pallas as pl
import jax.experimental.pallas.tpu as pltpu

F32 = jnp.float32
BF16 = jnp.bfloat16

S = 2048
D = 448
F = 1792
P2 = 2 * D
M = 512
NC = S // M
NS = M // 128
NG = M // 8
FT = 128
NT = F // FT
RB = 32
XS = 2
G2 = 5
B4 = 11
OSPLIT = 4
GELU_C1 = 0.7978845608028654
GELU_C2 = 0.7978845608028654 * 0.044715

S_VEC, S_BT, S_B0, S_B1, S_W0, S_W1, S_W2, S_OUT, S_X0 = range(9)
N_SEMS = S_X0 + XS


def _nt(a, b):
    return jax.lax.dot_general(a, b, (((1,), (1,)), ((), ())), preferred_element_type=F32)


def _kernel(xt_hbm, lre_hbm, lim_hbm, bre_hbm, bim_hbm, cre_hbm, cim_hbm, ldt_hbm, dsk_hbm,
            wg_hbm, wu_hbm, wdt_hbm, gw_hbm, o_hbm,
            xt_s, v0_s, v1_s, v2_s, v3_s, v4_s, bcat_s, wg_s, wu_s, wd_s, cre_s, cim_s, cp_s,
            const_s, hc_s, col_s, coef_s, o_s, xn_s, sems):
    vecs = (v0_s, v1_s, v2_s, v3_s, v4_s)

    def cp(src, dst, k):
        return pltpu.make_async_copy(src, dst, sems.at[k])

    def wait_all(group):
        for c in group:
            c.wait()

    fa = G2 * FT
    xw = M // XS
    g_vec = [cp(src, vecs[n], S_VEC)
             for n, src in enumerate((lre_hbm, lim_hbm, ldt_hbm, dsk_hbm, gw_hbm))]
    g_x0 = [[cp(xt_hbm.at[:, pl.ds(q * xw, xw)], xt_s.at[0, :, pl.ds(q * xw, xw)], S_X0 + q)]
            for q in range(XS)]
    g_bt = [cp(bre_hbm.at[pl.ds(384, 64), :], bcat_s.at[pl.ds(768, 64), :], S_BT),
            cp(bim_hbm.at[pl.ds(384, 64), :], bcat_s.at[pl.ds(832, 64), :], S_BT)]
    g_b0 = [cp(bre_hbm.at[pl.ds(0, 256), :], bcat_s.at[pl.ds(0, 256), :], S_B0)]
    g_b1 = [cp(bre_hbm.at[pl.ds(256, 128), :], bcat_s.at[pl.ds(256, 128), :], S_B1),
            cp(bim_hbm.at[pl.ds(0, 384), :], bcat_s.at[pl.ds(384, 384), :], S_B1)]
    g_w0 = [cp(wg_hbm.at[:, pl.ds(0, fa)], wg_s.at[:, pl.ds(0, fa)], S_W0),
            cp(wu_hbm.at[:, pl.ds(0, fa)], wu_s.at[:, pl.ds(0, fa)], S_W0)]
    g_w1 = [cp(wg_hbm.at[:, pl.ds(fa, F - fa)], wg_s.at[:, pl.ds(fa, F - fa)], S_W1),
            cp(wu_hbm.at[:, pl.ds(fa, F - fa)], wu_s.at[:, pl.ds(fa, F - fa)], S_W1)]
    g_w2 = [cp(wdt_hbm, wd_s, S_W2), cp(cre_hbm, cre_s, S_W2), cp(cim_hbm, cim_s, S_W2)]
    g_w2 += [cp(xt_hbm.at[:, pl.ds(i * M, M)], xt_s.at[i], S_W2) for i in range(1, NC)]

    def o_copy(i, s, r0, nr):
        return cp(o_s.at[i, pl.ds(r0, nr), pl.ds(s * 128, 128)],
                  o_hbm.at[pl.ds(r0, nr), pl.ds(i * M + s * 128, 128)], S_OUT)

    for group in [g_vec] + g_x0 + [g_bt, g_b0, g_b1, g_w0, g_w1, g_w2]:
        for c in group:
            c.start()

    wait_all(g_vec)

    def ext(v):
        return jnp.concatenate([v, v[:, 384:448]], axis=1)

    lre = vecs[0][...].astype(F32).reshape(1, D)
    lim = vecs[1][...].astype(F32).reshape(1, D)
    dt = jnp.exp(vecs[2][...].astype(F32).reshape(1, D)).astype(BF16).astype(F32)
    ar = dt * lre
    ai = dt * lim
    row = jax.lax.broadcasted_iota(jnp.int32, (8, 512), 0)
    lane = jax.lax.broadcasted_iota(jnp.int32, (8, 512), 1)
    k8 = (row + 1).astype(F32)
    mag = jnp.exp(k8 * ext(ar))
    ang = k8 * ext(ai)
    pr = mag * jnp.cos(ang)
    pi_ = mag * jnp.sin(ang) * jnp.where(lane >= D, -1.0, 1.0)
    const_s[0] = pr
    const_s[1] = pi_
    for n, kk in enumerate((1, 2, 4)):
        const_s[2 + 2 * n] = jnp.where(row >= kk, pr[kk - 1:kk, :], 0.0)
        const_s[3 + 2 * n] = jnp.where(row >= kk, pi_[kk - 1:kk, :], 0.0)
    hc_s[...] = jnp.zeros_like(hc_s)
    col_s[0] = jnp.broadcast_to(vecs[4][...].astype(F32).reshape(1, D), (128, D)).T
    col_s[1] = jnp.broadcast_to(vecs[3][...].astype(F32).reshape(1, D), (128, D)).T
    nre = pr[0:1, :D] - 1.0
    nim = pi_[0:1, :D]
    den = 1.0 / (lre * lre + lim * lim)
    coef_s[0] = jnp.broadcast_to(2.0 * ((nre * lre + nim * lim) * den), (8, D))
    coef_s[1] = jnp.broadcast_to(2.0 * ((nim * lre - nre * lim) * den), (8, D))

    def prep_c_block(r, cr8, ci8):
        rs = slice(r * 16, (r + 1) * 16)
        cr = jnp.concatenate([cr8, cr8], axis=0)
        ci = jnp.concatenate([ci8, ci8], axis=0)
        c_re = cre_s[rs, :].astype(F32)
        c_im = cim_s[rs, :].astype(F32)
        q_re = c_re * cr - c_im * ci
        q_im = -(c_re * ci + c_im * cr)
        cp_s[rs, 0:384] = q_re[:, 0:384].astype(BF16)
        cp_s[rs, 384:768] = q_im[:, 0:384].astype(BF16)
        cp_s[rs, 768:896] = jnp.concatenate(
            [q_re[:, 384:448], q_im[:, 384:448]], axis=1).astype(BF16)

    def zero_after(piece):
        z = jnp.where(piece[0:8, :] < -jnp.inf, 1.0, 0.0)
        return jnp.concatenate([z] * 4, axis=1)

    def chunk(i, first):
        if first:
            xs = []
            for q in range(XS):
                wait_all(g_x0[q])
                if q == XS - 1:
                    wait_all(g_bt)
                xs.append(xt_s[0, :, q * xw:(q + 1) * xw].T)
            x = jnp.concatenate(xs, axis=0)
        else:
            x = pltpu.bitcast(xn_s[...], BF16)
        v_t = _nt(x, bcat_s[768:896, :])
        if first:
            wait_all(g_b0)
        v_r0 = _nt(x, bcat_s[0:256, :])
        if first:
            wait_all(g_b1)
        v_r1 = _nt(x, bcat_s[256:384, :])
        v_im = _nt(x, bcat_s[384:768, :])
        v_re = jnp.concatenate([v_r0, v_r1], axis=1)
        if first:
            wait_all(g_w0)

        st = dict(c_re=hc_s[0], c_im=hc_s[1], g=0)
        hre, him = [], []

        def scan_group(z):
            gidx = st["g"]
            cs = [const_s[q] for q in range(8)]
            cs[2] = cs[2] + z
            cs[3] = cs[3] + z
            rs = slice(gidx * 8, gidx * 8 + 8)
            t = v_t[rs, :]
            vre = jnp.concatenate([v_re[rs, :], t], axis=1)
            vim = jnp.concatenate([v_im[rs, :], pltpu.roll(t, 64, 1)], axis=1)
            for n, kk in enumerate((1, 2, 4)):
                a_re, a_im = cs[2 + 2 * n], cs[3 + 2 * n]
                s_re = pltpu.roll(vre, kk, 0)
                s_im = pltpu.roll(vim, kk, 0)
                vre, vim = vre + (a_re * s_re - a_im * s_im), vim + (a_re * s_im + a_im * s_re)
            b_re = jnp.broadcast_to(st["c_re"][7:8, :], (8, 512))
            b_im = jnp.broadcast_to(st["c_im"][7:8, :], (8, 512))
            st["c_re"] = vre + (cs[0] * b_re - cs[1] * b_im)
            st["c_im"] = vim + (cs[0] * b_im + cs[1] * b_re)
            hre.append(st["c_re"])
            him.append(st["c_im"])
            st["g"] = gidx + 1

        hhs = []
        per = -(-NG // NT)
        npc = M // RB
        cblk = 0
        for j in range(NT):
            if first and j == G2:
                wait_all(g_w1)
            if first and j == B4:
                wait_all(g_w2)
            g = jnp.dot(x, wg_s[:, j * FT:(j + 1) * FT], preferred_element_type=F32)
            u = jnp.dot(x, wu_s[:, j * FT:(j + 1) * FT], preferred_element_type=F32)
            ng_here = min(per, NG - st["g"])
            g_trig = [(q * npc) // ng_here for q in range(ng_here)]
            c_trig = []
            if first and j >= B4:
                nblk = -(-(D // 16 - cblk) // (NT - j))
                c_trig = [((2 * q + 1) * npc) // (2 * nblk) for q in range(nblk)]
            pieces = []
            for rb in range(npc):
                rs = slice(rb * RB, (rb + 1) * RB)
                gg = g[rs, :]
                inner = gg * (GELU_C1 + GELU_C2 * (gg * gg))
                r = (0.5 * gg) * u[rs, :]
                pieces.append(r + r * jnp.tanh(inner))
                if rb in g_trig or rb in c_trig:
                    z = zero_after(pieces[-1])
                    for _ in range(g_trig.count(rb)):
                        scan_group(z)
                    for _ in range(c_trig.count(rb)):
                        prep_c_block(cblk, coef_s[0] + z[:, :D], coef_s[1] + z[:, :D])
                        cblk += 1
            hhs.append(jnp.concatenate(pieces, axis=0))
            if j >= B4:
                nxt = jnp.minimum(i + 1, NC - 1)
                for q in range(NS):
                    if B4 + (q * (NT - B4)) // NS == j:
                        xq = xt_s[nxt, :, q * 128:(q + 1) * 128].T
                        xn_s[q * 64:(q + 1) * 64, :] = pltpu.bitcast(xq, jnp.uint32)
        assert st["g"] == NG and cblk == (D // 16 if first else 0)
        hc_s[0] = st["c_re"]
        hc_s[1] = st["c_im"]
        h_re = jnp.concatenate(hre, axis=0)
        h_im = jnp.concatenate(him, axis=0)
        hp = jnp.concatenate([h_re[:, :384], h_im[:, :384], h_re[:, 384:]], axis=1)
        hh = jnp.concatenate(hhs, axis=1)

        for s in range(NS):
            sl = slice(s * 128, (s + 1) * 128)
            xtf = xt_s[i, :, sl].astype(F32)
            a = _nt(cp_s[...], hp[sl, :].astype(BF16)) + xtf * col_s[1]
            b = _nt(wd_s[...], hh[sl, :].astype(BF16))
            gate = jax.nn.sigmoid(jnp.sum(xtf * col_s[0], axis=0, keepdims=True))
            nsp = OSPLIT if s == NS - 1 else 1
            nr = D // nsp
            for q in range(nsp):
                rr = slice(q * nr, (q + 1) * nr)
                o_s[i, rr, sl] = b[rr, :] + gate * (a[rr, :] - b[rr, :])
                o_copy(i, s, q * nr, nr).start()

    chunk(0, True)

    def body(i, carry):
        chunk(i, False)
        return carry

    jax.lax.fori_loop(1, NC, body, 0)
    pltpu.make_async_copy(o_s, o_s, sems.at[S_OUT]).wait()


@jax.jit
def pallas_gated_mix__ssm_conv_s5__glu_gated_geglu__prompt_kernel(
    A_x: jax.Array,
    A_Lambda_re: jax.Array,
    A_Lambda_im: jax.Array,
    A_B_re: jax.Array,
    A_B_im: jax.Array,
    A_C_re: jax.Array,
    A_C_im: jax.Array,
    A_log_dt: jax.Array,
    A_Dskip: jax.Array,
    B_x: jax.Array,
    B_w_gate: jax.Array,
    B_w_up: jax.Array,
    B_w_down: jax.Array,
    gate_w: jax.Array,
):
    del B_x
    assert A_x.shape == (1, S, D) and B_w_gate.shape == (D, F) and B_w_down.shape == (F, D)
    xt = jnp.transpose(A_x.reshape(S, D))
    wdt = jnp.transpose(B_w_down)
    hbm = pl.BlockSpec(memory_space=pl.ANY)
    out_t = pl.pallas_call(
        _kernel,
        in_specs=[hbm] * 13,
        out_specs=hbm,
        out_shape=jax.ShapeDtypeStruct((D, S), F32),
        scratch_shapes=[
            pltpu.VMEM((NC, D, M), BF16),
            pltpu.VMEM((D,), BF16), pltpu.VMEM((D,), BF16), pltpu.VMEM((D,), BF16),
            pltpu.VMEM((D,), BF16), pltpu.VMEM((D,), BF16),
            pltpu.VMEM((P2, D), BF16),
            pltpu.VMEM((D, F), BF16),
            pltpu.VMEM((D, F), BF16),
            pltpu.VMEM((D, F), BF16),
            pltpu.VMEM((D, D), BF16),
            pltpu.VMEM((D, D), BF16),
            pltpu.VMEM((D, P2), BF16),
            pltpu.VMEM((8, 8, 512), F32),
            pltpu.VMEM((2, 8, 512), F32),
            pltpu.VMEM((2, D, 128), F32),
            pltpu.VMEM((2, 8, D), F32),
            pltpu.VMEM((NC, D, M), F32),
            pltpu.VMEM((M // 2, D), jnp.uint32),
            pltpu.SemaphoreType.DMA((N_SEMS,)),
        ],
        compiler_params=pltpu.CompilerParams(vmem_limit_bytes=100 * 1024 * 1024),
    )(xt, A_Lambda_re, A_Lambda_im, A_B_re, A_B_im, A_C_re, A_C_im, A_log_dt, A_Dskip,
      B_w_gate, B_w_up, wdt, gate_w)
    return jnp.transpose(out_t).reshape(1, S, D)
```

```python
import functools

import jax
import jax.numpy as jnp
import jax.experimental.pallas as pl
import jax.experimental.pallas.tpu as pltpu

F32 = jnp.float32
BF16 = jnp.bfloat16

S = 2048
D = 448
F = 1792
P2 = 2 * D
M = 512
NC = S // M
NS = M // 128
NG = M // 8
FT = 128
NT = F // FT
RB = 32
XS = 2
G2 = 5
B4 = 11
OSPLIT = 4
GELU_C1 = 0.7978845608028654
GELU_C2 = 0.7978845608028654 * 0.044715

S_VEC, S_BT, S_B0, S_B1, S_W0, S_W1, S_W2, S_OUT, S_X0 = range(9)
N_SEMS = S_X0 + XS


def _nt(a, b):
    return jax.lax.dot_general(a, b, (((1,), (1,)), ((), ())), preferred_element_type=F32)


def _kernel(xt_hbm, lre_hbm, lim_hbm, bre_hbm, bim_hbm, cre_hbm, cim_hbm, ldt_hbm, dsk_hbm,
            wg_hbm, wu_hbm, wdt_hbm, gw_hbm, o_hbm,
            xt_s, v0_s, v1_s, v2_s, v3_s, v4_s, bcat_s, wg_s, wu_s, wd_s, cre_s, cim_s, cp_s,
            const_s, hc_s, col_s, coef_s, o_s, xn_s, sems):
    vecs = (v0_s, v1_s, v2_s, v3_s, v4_s)

    def cp(src, dst, k):
        return pltpu.make_async_copy(src, dst, sems.at[k])

    def wait_all(group):
        for c in group:
            c.wait()

    fa = G2 * FT
    xw = M // XS
    g_vec = [cp(src, vecs[n], S_VEC)
             for n, src in enumerate((lre_hbm, lim_hbm, ldt_hbm, dsk_hbm, gw_hbm))]
    g_x0 = [[cp(xt_hbm.at[:, pl.ds(q * xw, xw)], xt_s.at[0, :, pl.ds(q * xw, xw)], S_X0 + q)]
            for q in range(XS)]
    g_bt = [cp(bre_hbm.at[pl.ds(384, 64), :], bcat_s.at[pl.ds(768, 64), :], S_BT),
            cp(bim_hbm.at[pl.ds(384, 64), :], bcat_s.at[pl.ds(832, 64), :], S_BT)]
    g_b0 = [cp(bre_hbm.at[pl.ds(0, 256), :], bcat_s.at[pl.ds(0, 256), :], S_B0)]
    g_b1 = [cp(bre_hbm.at[pl.ds(256, 128), :], bcat_s.at[pl.ds(256, 128), :], S_B1),
            cp(bim_hbm.at[pl.ds(0, 384), :], bcat_s.at[pl.ds(384, 384), :], S_B1)]
    g_w0 = [cp(wg_hbm.at[:, pl.ds(0, fa)], wg_s.at[:, pl.ds(0, fa)], S_W0),
            cp(wu_hbm.at[:, pl.ds(0, fa)], wu_s.at[:, pl.ds(0, fa)], S_W0)]
    g_w1 = [cp(wg_hbm.at[:, pl.ds(fa, F - fa)], wg_s.at[:, pl.ds(fa, F - fa)], S_W1),
            cp(wu_hbm.at[:, pl.ds(fa, F - fa)], wu_s.at[:, pl.ds(fa, F - fa)], S_W1)]
    g_w2 = [cp(wdt_hbm, wd_s, S_W2), cp(cre_hbm, cre_s, S_W2), cp(cim_hbm, cim_s, S_W2)]
    g_w2 += [cp(xt_hbm.at[:, pl.ds(i * M, M)], xt_s.at[i], S_W2) for i in range(1, NC)]

    def o_copy(i, s, r0, nr):
        return cp(o_s.at[i, pl.ds(r0, nr), pl.ds(s * 128, 128)],
                  o_hbm.at[pl.ds(r0, nr), pl.ds(i * M + s * 128, 128)], S_OUT)

    for group in [g_vec] + g_x0 + [g_bt, g_b0, g_b1, g_w0, g_w1, g_w2]:
        for c in group:
            c.start()

    wait_all(g_vec)

    def ext(v):
        return jnp.concatenate([v, v[:, 384:448]], axis=1)

    lre = vecs[0][...].astype(F32).reshape(1, D)
    lim = vecs[1][...].astype(F32).reshape(1, D)
    dt = jnp.exp(vecs[2][...].astype(F32).reshape(1, D)).astype(BF16).astype(F32)
    ar = dt * lre
    ai = dt * lim
    row = jax.lax.broadcasted_iota(jnp.int32, (8, 512), 0)
    lane = jax.lax.broadcasted_iota(jnp.int32, (8, 512), 1)
    k8 = (row + 1).astype(F32)
    mag = jnp.exp(k8 * ext(ar))
    ang = k8 * ext(ai)
    pr = mag * jnp.cos(ang)
    pi_ = mag * jnp.sin(ang) * jnp.where(lane >= D, -1.0, 1.0)
    const_s[0] = pr
    const_s[1] = pi_
    for n, kk in enumerate((1, 2, 4)):
        const_s[2 + 2 * n] = jnp.where(row >= kk, pr[kk - 1:kk, :], 0.0)
        const_s[3 + 2 * n] = jnp.where(row >= kk, pi_[kk - 1:kk, :], 0.0)
    hc_s[...] = jnp.zeros_like(hc_s)
    col_s[0] = jnp.broadcast_to(vecs[4][...].astype(F32).reshape(1, D), (128, D)).T
    col_s[1] = jnp.broadcast_to(vecs[3][...].astype(F32).reshape(1, D), (128, D)).T
    nre = pr[0:1, :D] - 1.0
    nim = pi_[0:1, :D]
    den = 1.0 / (lre * lre + lim * lim)
    coef_s[0] = jnp.broadcast_to(2.0 * ((nre * lre + nim * lim) * den), (8, D))
    coef_s[1] = jnp.broadcast_to(2.0 * ((nim * lre - nre * lim) * den), (8, D))

    def prep_c_block(r, cr8, ci8):
        rs = slice(r * 16, (r + 1) * 16)
        cr = jnp.concatenate([cr8, cr8], axis=0)
        ci = jnp.concatenate([ci8, ci8], axis=0)
        c_re = cre_s[rs, :].astype(F32)
        c_im = cim_s[rs, :].astype(F32)
        q_re = c_re * cr - c_im * ci
        q_im = -(c_re * ci + c_im * cr)
        cp_s[rs, 0:384] = q_re[:, 0:384].astype(BF16)
        cp_s[rs, 384:768] = q_im[:, 0:384].astype(BF16)
        cp_s[rs, 768:896] = jnp.concatenate(
            [q_re[:, 384:448], q_im[:, 384:448]], axis=1).astype(BF16)

    def zero_after(piece):
        z = jnp.where(piece[0:8, :] < -jnp.inf, 1.0, 0.0)
        return jnp.concatenate([z] * 4, axis=1)

    def chunk(i, first):
        if first:
            xs = []
            for q in range(XS):
                wait_all(g_x0[q])
                if q == XS - 1:
                    wait_all(g_bt)
                xs.append(xt_s[0, :, q * xw:(q + 1) * xw].T)
            x = jnp.concatenate(xs, axis=0)
        else:
            x = pltpu.bitcast(xn_s[...], BF16)
            g_first = jnp.dot(x, wg_s[:, 0:FT], preferred_element_type=F32)
        v_t = _nt(x, bcat_s[768:896, :])
        if first:
            wait_all(g_b0)
        v_r0 = _nt(x, bcat_s[0:256, :])
        if first:
            wait_all(g_b1)
        v_r1 = _nt(x, bcat_s[256:384, :])
        v_im = _nt(x, bcat_s[384:768, :])
        v_re = jnp.concatenate([v_r0, v_r1], axis=1)
        if first:
            wait_all(g_w0)

        st = dict(c_re=hc_s[0], c_im=hc_s[1], g=0)
        hre, him = [], []

        def scan_group(z):
            gidx = st["g"]
            cs = [const_s[q] for q in range(8)]
            cs[2] = cs[2] + z
            cs[3] = cs[3] + z
            rs = slice(gidx * 8, gidx * 8 + 8)
            t = v_t[rs, :]
            vre = jnp.concatenate([v_re[rs, :], t], axis=1)
            vim = jnp.concatenate([v_im[rs, :], pltpu.roll(t, 64, 1)], axis=1)
            for n, kk in enumerate((1, 2, 4)):
                a_re, a_im = cs[2 + 2 * n], cs[3 + 2 * n]
                s_re = pltpu.roll(vre, kk, 0)
                s_im = pltpu.roll(vim, kk, 0)
                vre, vim = vre + (a_re * s_re - a_im * s_im), vim + (a_re * s_im + a_im * s_re)
            b_re = jnp.broadcast_to(st["c_re"][7:8, :], (8, 512))
            b_im = jnp.broadcast_to(st["c_im"][7:8, :], (8, 512))
            st["c_re"] = vre + (cs[0] * b_re - cs[1] * b_im)
            st["c_im"] = vim + (cs[0] * b_im + cs[1] * b_re)
            hre.append(st["c_re"])
            him.append(st["c_im"])
            st["g"] = gidx + 1

        hhs = []
        per = -(-NG // NT)
        npc = M // RB
        cblk = 0
        for j in range(NT):
            if first and j == G2:
                wait_all(g_w1)
            if first and j == B4:
                wait_all(g_w2)
            if j == 0 and not first:
                g = g_first
            else:
                g = jnp.dot(x, wg_s[:, j * FT:(j + 1) * FT], preferred_element_type=F32)
            u = jnp.dot(x, wu_s[:, j * FT:(j + 1) * FT], preferred_element_type=F32)
            ng_here = min(per, NG - st["g"])
            g_trig = [(q * npc) // ng_here for q in range(ng_here)]
            c_trig = []
            if first and j >= B4:
                nblk = -(-(D // 16 - cblk) // (NT - j))
                c_trig = [((2 * q + 1) * npc) // (2 * nblk) for q in range(nblk)]
            pieces = []
            for rb in range(npc):
                rs = slice(rb * RB, (rb + 1) * RB)
                gg = g[rs, :]
                inner = gg * (GELU_C1 + GELU_C2 * (gg * gg))
                r = gg * u[rs, :]
                pieces.append(r + r * jnp.tanh(inner))
                if rb in g_trig or rb in c_trig:
                    z = zero_after(pieces[-1])
                    for _ in range(g_trig.count(rb)):
                        scan_group(z)
                    for _ in range(c_trig.count(rb)):
                        prep_c_block(cblk, coef_s[0] + z[:, :D], coef_s[1] + z[:, :D])
                        cblk += 1
            hhs.append(jnp.concatenate(pieces, axis=0))
            if j >= B4:
                nxt = jnp.minimum(i + 1, NC - 1)
                for q in range(NS):
                    if B4 + (q * (NT - B4)) // NS == j:
                        xq = xt_s[nxt, :, q * 128:(q + 1) * 128].T
                        xn_s[q * 64:(q + 1) * 64, :] = pltpu.bitcast(xq, jnp.uint32)
        assert st["g"] == NG and cblk == (D // 16 if first else 0)
        hc_s[0] = st["c_re"]
        hc_s[1] = st["c_im"]
        h_re = jnp.concatenate(hre, axis=0)
        h_im = jnp.concatenate(him, axis=0)
        hp = jnp.concatenate([h_re[:, :384], h_im[:, :384], h_re[:, 384:]], axis=1)
        hh = jnp.concatenate(hhs, axis=1)

        for s in range(NS):
            sl = slice(s * 128, (s + 1) * 128)
            xtf = xt_s[i, :, sl].astype(F32)
            a = _nt(cp_s[...], hp[sl, :].astype(BF16)) + xtf * col_s[1]
            b = _nt(wd_s[...], hh[sl, :].astype(BF16))
            gate = jax.nn.sigmoid(jnp.sum(xtf * col_s[0], axis=0, keepdims=True))
            g1 = 0.5 * (1.0 - gate)
            nsp = OSPLIT if s == NS - 1 else 1
            nr = D // nsp
            for q in range(nsp):
                rr = slice(q * nr, (q + 1) * nr)
                o_s[i, rr, sl] = gate * a[rr, :] + g1 * b[rr, :]
                o_copy(i, s, q * nr, nr).start()

    chunk(0, True)

    def body(i, carry):
        chunk(i, False)
        return carry

    jax.lax.fori_loop(1, NC, body, 0)
    pltpu.make_async_copy(o_s, o_s, sems.at[S_OUT]).wait()


@jax.jit
def pallas_gated_mix__ssm_conv_s5__glu_gated_geglu__prompt_kernel(
    A_x: jax.Array,
    A_Lambda_re: jax.Array,
    A_Lambda_im: jax.Array,
    A_B_re: jax.Array,
    A_B_im: jax.Array,
    A_C_re: jax.Array,
    A_C_im: jax.Array,
    A_log_dt: jax.Array,
    A_Dskip: jax.Array,
    B_x: jax.Array,
    B_w_gate: jax.Array,
    B_w_up: jax.Array,
    B_w_down: jax.Array,
    gate_w: jax.Array,
):
    del B_x
    assert A_x.shape == (1, S, D) and B_w_gate.shape == (D, F) and B_w_down.shape == (F, D)
    xt = jnp.transpose(A_x.reshape(S, D))
    wdt = jnp.transpose(B_w_down)
    hbm = pl.BlockSpec(memory_space=pl.ANY)
    out_t = pl.pallas_call(
        _kernel,
        in_specs=[hbm] * 13,
        out_specs=hbm,
        out_shape=jax.ShapeDtypeStruct((D, S), F32),
        scratch_shapes=[
            pltpu.VMEM((NC, D, M), BF16),
            pltpu.VMEM((D,), BF16), pltpu.VMEM((D,), BF16), pltpu.VMEM((D,), BF16),
            pltpu.VMEM((D,), BF16), pltpu.VMEM((D,), BF16),
            pltpu.VMEM((P2, D), BF16),
            pltpu.VMEM((D, F), BF16),
            pltpu.VMEM((D, F), BF16),
            pltpu.VMEM((D, F), BF16),
            pltpu.VMEM((D, D), BF16),
            pltpu.VMEM((D, D), BF16),
            pltpu.VMEM((D, P2), BF16),
            pltpu.VMEM((8, 8, 512), F32),
            pltpu.VMEM((2, 8, 512), F32),
            pltpu.VMEM((2, D, 128), F32),
            pltpu.VMEM((2, 8, D), F32),
            pltpu.VMEM((NC, D, M), F32),
            pltpu.VMEM((M // 2, D), jnp.uint32),
            pltpu.SemaphoreType.DMA((N_SEMS,)),
        ],
        compiler_params=pltpu.CompilerParams(vmem_limit_bytes=100 * 1024 * 1024),
    )(xt, A_Lambda_re, A_Lambda_im, A_B_re, A_B_im, A_C_re, A_C_im, A_log_dt, A_Dskip,
      B_w_gate, B_w_up, wdt, gate_w)
    return jnp.transpose(out_t).reshape(1, S, D)
```

```python
import jax
import jax.numpy as jnp
import jax.experimental.pallas as pl
import jax.experimental.pallas.tpu as pltpu

F32 = jnp.float32
BF16 = jnp.bfloat16

S = 2048
D = 448
F = 1792
P2 = 2 * D
M = 512
NC = S // M
NS = M // 128
NG = M // 8
FT = 128
NT = F // FT
RB = 32
G2 = 5
B4 = 11
OSPLIT = 4
GELU_C1 = 0.7978845608028654
GELU_C2 = 0.7978845608028654 * 0.044715

S_VEC = S_B1 = S_OUT = 0
S_XA = S_W0 = 1
S_XB = S_W1 = 2
S_B0 = S_W2 = 3
N_SEMS = 4


def _nt(a, b):
    return jax.lax.dot_general(a, b, (((1,), (1,)), ((), ())), preferred_element_type=F32)


def _kernel(xt_hbm, lre_hbm, lim_hbm, bre_hbm, bim_hbm, cre_hbm, cim_hbm, ldt_hbm, dsk_hbm,
            wg_hbm, wu_hbm, wdt_hbm, gw_hbm, o_hbm,
            xt_s, v0_s, v1_s, v2_s, v3_s, v4_s, bcat_s, wg_s, wu_s, wd_s, cre_s, cim_s, cp_s,
            const_s, hc_s, col_s, coef_s, o_s, xn_s, sems):
    vecs = (v0_s, v1_s, v2_s, v3_s, v4_s)

    def cp(src, dst, k):
        return pltpu.make_async_copy(src, dst, sems.at[k])

    def wait_all(group):
        for c in group:
            c.wait()

    fa = G2 * FT
    xw = M // 2
    g_vec = [cp(src, vecs[n], S_VEC)
             for n, src in enumerate((lre_hbm, lim_hbm, ldt_hbm, dsk_hbm, gw_hbm))]
    g_xa = [cp(xt_hbm.at[:, pl.ds(0, xw)], xt_s.at[0, :, pl.ds(0, xw)], S_XA)]
    g_xb = [cp(xt_hbm.at[:, pl.ds(xw, xw)], xt_s.at[0, :, pl.ds(xw, xw)], S_XB)]
    g_xb += [cp(bre_hbm.at[pl.ds(384, 64), :], bcat_s.at[pl.ds(768, 64), :], S_XB),
             cp(bim_hbm.at[pl.ds(384, 64), :], bcat_s.at[pl.ds(832, 64), :], S_XB)]
    g_b0 = [cp(bre_hbm.at[pl.ds(0, 256), :], bcat_s.at[pl.ds(0, 256), :], S_B0)]
    g_b1 = [cp(bre_hbm.at[pl.ds(256, 128), :], bcat_s.at[pl.ds(256, 128), :], S_B1),
            cp(bim_hbm.at[pl.ds(0, 384), :], bcat_s.at[pl.ds(384, 384), :], S_B1)]
    g_w0 = [cp(wg_hbm.at[:, pl.ds(0, fa)], wg_s.at[:, pl.ds(0, fa)], S_W0),
            cp(wu_hbm.at[:, pl.ds(0, fa)], wu_s.at[:, pl.ds(0, fa)], S_W0)]
    g_w1 = [cp(wg_hbm.at[:, pl.ds(fa, F - fa)], wg_s.at[:, pl.ds(fa, F - fa)], S_W1),
            cp(wu_hbm.at[:, pl.ds(fa, F - fa)], wu_s.at[:, pl.ds(fa, F - fa)], S_W1)]
    g_w2 = [cp(wdt_hbm, wd_s, S_W2), cp(cre_hbm, cre_s, S_W2), cp(cim_hbm, cim_s, S_W2)]
    g_w2 += [cp(xt_hbm.at[:, pl.ds(i * M, M)], xt_s.at[i], S_W2) for i in range(1, NC)]

    def o_copy(i, s, r0, nr):
        return cp(o_s.at[i, pl.ds(r0, nr), pl.ds(s * 128, 128)],
                  o_hbm.at[pl.ds(r0, nr), pl.ds(i * M + s * 128, 128)], S_OUT)

    def start_all(group):
        for c in group:
            c.start()

    for group in (g_vec, g_xa, g_xb, g_b0):
        start_all(group)

    wait_all(g_vec)
    start_all(g_b1)

    def ext(v):
        return jnp.concatenate([v, v[:, 384:448]], axis=1)

    lre = vecs[0][...].astype(F32).reshape(1, D)
    lim = vecs[1][...].astype(F32).reshape(1, D)
    dt = jnp.exp(vecs[2][...].astype(F32).reshape(1, D)).astype(BF16).astype(F32)
    ar = dt * lre
    ai = dt * lim
    row = jax.lax.broadcasted_iota(jnp.int32, (8, 512), 0)
    lane = jax.lax.broadcasted_iota(jnp.int32, (8, 512), 1)
    k8 = (row + 1).astype(F32)
    mag = jnp.exp(k8 * ext(ar))
    ang = k8 * ext(ai)
    pr = mag * jnp.cos(ang)
    pi_ = mag * jnp.sin(ang) * jnp.where(lane >= D, -1.0, 1.0)
    const_s[0] = pr
    const_s[1] = pi_
    for n, kk in enumerate((1, 2, 4)):
        const_s[2 + 2 * n] = jnp.where(row >= kk, pr[kk - 1:kk, :], 0.0)
        const_s[3 + 2 * n] = jnp.where(row >= kk, pi_[kk - 1:kk, :], 0.0)
    hc_s[...] = jnp.zeros_like(hc_s)
    col_s[0] = jnp.broadcast_to(vecs[4][...].astype(F32).reshape(1, D), (128, D)).T
    col_s[1] = jnp.broadcast_to(vecs[3][...].astype(F32).reshape(1, D), (128, D)).T
    nre = pr[0:1, :D] - 1.0
    nim = pi_[0:1, :D]
    den = 1.0 / (lre * lre + lim * lim)
    coef_s[0] = jnp.broadcast_to(2.0 * ((nre * lre + nim * lim) * den), (8, D))
    coef_s[1] = jnp.broadcast_to(2.0 * ((nim * lre - nre * lim) * den), (8, D))

    def prep_c_block(r, cr8, ci8):
        rs = slice(r * 16, (r + 1) * 16)
        cr = jnp.concatenate([cr8, cr8], axis=0)
        ci = jnp.concatenate([ci8, ci8], axis=0)
        c_re = cre_s[rs, :].astype(F32)
        c_im = cim_s[rs, :].astype(F32)
        q_re = c_re * cr - c_im * ci
        q_im = -(c_re * ci + c_im * cr)
        cp_s[rs, 0:384] = q_re[:, 0:384].astype(BF16)
        cp_s[rs, 384:768] = q_im[:, 0:384].astype(BF16)
        cp_s[rs, 768:896] = jnp.concatenate(
            [q_re[:, 384:448], q_im[:, 384:448]], axis=1).astype(BF16)

    def zero_after(piece):
        z = jnp.where(piece[0:8, :] < -jnp.inf, 1.0, 0.0)
        return jnp.concatenate([z] * 4, axis=1)

    def chunk(i, first):
        if first:
            wait_all(g_xa)
            start_all(g_w0)
            xa = xt_s[0, :, 0:xw].T
            wait_all(g_xb)
            start_all(g_w1)
            x = jnp.concatenate([xa, xt_s[0, :, xw:M].T], axis=0)
        else:
            x = pltpu.bitcast(xn_s[...], BF16)
            g_first = jnp.dot(x, wg_s[:, 0:FT], preferred_element_type=F32)
        v_t = _nt(x, bcat_s[768:896, :])
        if first:
            wait_all(g_b0)
            start_all(g_w2)
        v_r0 = _nt(x, bcat_s[0:256, :])
        if first:
            wait_all(g_b1)
        v_r1 = _nt(x, bcat_s[256:384, :])
        v_im = _nt(x, bcat_s[384:768, :])
        v_re = jnp.concatenate([v_r0, v_r1], axis=1)
        if first:
            wait_all(g_w0)

        st = dict(c_re=hc_s[0], c_im=hc_s[1], g=0)
        hre, him = [], []

        def scan_group(z):
            gidx = st["g"]
            cs = [const_s[q] for q in range(8)]
            cs[2] = cs[2] + z
            cs[3] = cs[3] + z
            rs = slice(gidx * 8, gidx * 8 + 8)
            t = v_t[rs, :]
            vre = jnp.concatenate([v_re[rs, :], t], axis=1)
            vim = jnp.concatenate([v_im[rs, :], pltpu.roll(t, 64, 1)], axis=1)
            for n, kk in enumerate((1, 2, 4)):
                a_re, a_im = cs[2 + 2 * n], cs[3 + 2 * n]
                s_re = pltpu.roll(vre, kk, 0)
                s_im = pltpu.roll(vim, kk, 0)
                vre, vim = vre + (a_re * s_re - a_im * s_im), vim + (a_re * s_im + a_im * s_re)
            b_re = jnp.broadcast_to(st["c_re"][7:8, :], (8, 512))
            b_im = jnp.broadcast_to(st["c_im"][7:8, :], (8, 512))
            st["c_re"] = vre + (cs[0] * b_re - cs[1] * b_im)
            st["c_im"] = vim + (cs[0] * b_im + cs[1] * b_re)
            hre.append(st["c_re"])
            him.append(st["c_im"])
            st["g"] = gidx + 1

        hhs = []
        per = -(-NG // NT)
        npc = M // RB
        cblk = 0
        for j in range(NT):
            if first and j == G2:
                wait_all(g_w1)
            if first and j == B4:
                wait_all(g_w2)
            if j == 0 and not first:
                g = g_first
            else:
                g = jnp.dot(x, wg_s[:, j * FT:(j + 1) * FT], preferred_element_type=F32)
            u = jnp.dot(x, wu_s[:, j * FT:(j + 1) * FT], preferred_element_type=F32)
            ng_here = min(per, NG - st["g"])
            g_trig = [(q * npc) // ng_here for q in range(ng_here)]
            c_trig = []
            if first and j >= B4:
                nblk = -(-(D // 16 - cblk) // (NT - j))
                c_trig = [((2 * q + 1) * npc) // (2 * nblk) for q in range(nblk)]
            pieces = []
            for rb in range(npc):
                rs = slice(rb * RB, (rb + 1) * RB)
                gg = g[rs, :]
                inner = gg * (GELU_C1 + GELU_C2 * (gg * gg))
                r = gg * u[rs, :]
                pieces.append(r + r * jnp.tanh(inner))
                if rb in g_trig or rb in c_trig:
                    z = zero_after(pieces[-1])
                    for _ in range(g_trig.count(rb)):
                        scan_group(z)
                    for _ in range(c_trig.count(rb)):
                        prep_c_block(cblk, coef_s[0] + z[:, :D], coef_s[1] + z[:, :D])
                        cblk += 1
            hhs.append(jnp.concatenate(pieces, axis=0))
            if j >= B4:
                nxt = jnp.minimum(i + 1, NC - 1)
                for q in range(NS):
                    if B4 + (q * (NT - B4)) // NS == j:
                        xq = xt_s[nxt, :, q * 128:(q + 1) * 128].T
                        xn_s[q * 64:(q + 1) * 64, :] = pltpu.bitcast(xq, jnp.uint32)
        assert st["g"] == NG and cblk == (D // 16 if first else 0)
        hc_s[0] = st["c_re"]
        hc_s[1] = st["c_im"]
        h_re = jnp.concatenate(hre, axis=0)
        h_im = jnp.concatenate(him, axis=0)
        hp = jnp.concatenate([h_re[:, :384], h_im[:, :384], h_re[:, 384:]], axis=1)
        hh = jnp.concatenate(hhs, axis=1)

        for s in range(NS):
            sl = slice(s * 128, (s + 1) * 128)
            xtf = xt_s[i, :, sl].astype(F32)
            a = _nt(cp_s[...], hp[sl, :].astype(BF16)) + xtf * col_s[1]
            b = _nt(wd_s[...], hh[sl, :].astype(BF16))
            gate = jax.nn.sigmoid(jnp.sum(xtf * col_s[0], axis=0, keepdims=True))
            g1 = 0.5 * (1.0 - gate)
            nsp = OSPLIT if s == NS - 1 else 1
            nr = D // nsp
            for q in range(nsp):
                rr = slice(q * nr, (q + 1) * nr)
                o_s[i, rr, sl] = gate * a[rr, :] + g1 * b[rr, :]
                o_copy(i, s, q * nr, nr).start()

    chunk(0, True)

    def body(i, carry):
        chunk(i, False)
        return carry

    jax.lax.fori_loop(1, NC, body, 0)
    pltpu.make_async_copy(o_s, o_s, sems.at[S_OUT]).wait()


@jax.jit
def pallas_gated_mix__ssm_conv_s5__glu_gated_geglu__prompt_kernel(
    A_x: jax.Array,
    A_Lambda_re: jax.Array,
    A_Lambda_im: jax.Array,
    A_B_re: jax.Array,
    A_B_im: jax.Array,
    A_C_re: jax.Array,
    A_C_im: jax.Array,
    A_log_dt: jax.Array,
    A_Dskip: jax.Array,
    B_x: jax.Array,
    B_w_gate: jax.Array,
    B_w_up: jax.Array,
    B_w_down: jax.Array,
    gate_w: jax.Array,
):
    del B_x
    assert A_x.shape == (1, S, D) and B_w_gate.shape == (D, F) and B_w_down.shape == (F, D)
    xt = jnp.transpose(A_x.reshape(S, D))
    wdt = jnp.transpose(B_w_down)
    hbm = pl.BlockSpec(memory_space=pl.ANY)
    out_t = pl.pallas_call(
        _kernel,
        in_specs=[hbm] * 13,
        out_specs=hbm,
        out_shape=jax.ShapeDtypeStruct((D, S), F32),
        scratch_shapes=[
            pltpu.VMEM((NC, D, M), BF16),
            pltpu.VMEM((D,), BF16), pltpu.VMEM((D,), BF16), pltpu.VMEM((D,), BF16),
            pltpu.VMEM((D,), BF16), pltpu.VMEM((D,), BF16),
            pltpu.VMEM((P2, D), BF16),
            pltpu.VMEM((D, F), BF16),
            pltpu.VMEM((D, F), BF16),
            pltpu.VMEM((D, F), BF16),
            pltpu.VMEM((D, D), BF16),
            pltpu.VMEM((D, D), BF16),
            pltpu.VMEM((D, P2), BF16),
            pltpu.VMEM((8, 8, 512), F32),
            pltpu.VMEM((2, 8, 512), F32),
            pltpu.VMEM((2, D, 128), F32),
            pltpu.VMEM((2, 8, D), F32),
            pltpu.VMEM((NC, D, M), F32),
            pltpu.VMEM((M // 2, D), jnp.uint32),
            pltpu.SemaphoreType.DMA((N_SEMS,)),
        ],
        compiler_params=pltpu.CompilerParams(vmem_limit_bytes=100 * 1024 * 1024),
    )(xt, A_Lambda_re, A_Lambda_im, A_B_re, A_B_im, A_C_re, A_C_im, A_log_dt, A_Dskip,
      B_w_gate, B_w_up, wdt, gate_w)
    return jnp.transpose(out_t).reshape(1, S, D)
```

```python
import jax
import jax.numpy as jnp
import jax.experimental.pallas as pl
import jax.experimental.pallas.tpu as pltpu

F32 = jnp.float32
BF16 = jnp.bfloat16

S = 2048
D = 448
F = 1792
P2 = 2 * D
M = 512
NC = S // M
NS = M // 128
NG = M // 8
FT = 128
NT = F // FT
RB = 32
T_W1 = 4
T_WC = 8
T_W2 = 12
T_PC = 9
T_PF = 9
PIN_EARLY = 48
PIN_ROW = 288
PIN_PIECE = 8
PAD = 16
OSPLIT = 4
GELU_C1 = 0.7978845608028654
GELU_C2 = 0.7978845608028654 * 0.044715

S_VEC = S_B0 = S_W1 = 0
S_XA = S_B1 = S_WC = 1
S_XB = S_W0 = S_OUT = 2
S_BT = S_B2 = S_W2 = 3
N_SEMS = 4


def _nt(a, b):
    return jax.lax.dot_general(a, b, (((1,), (1,)), ((), ())), preferred_element_type=F32)


def _kernel(xt_hbm, lre_hbm, lim_hbm, bre_hbm, bim_hbm, cre_hbm, cim_hbm, ldt_hbm, dsk_hbm,
            wg_hbm, wu_hbm, wdt_hbm, gw_hbm, o_hbm,
            xt_s, v0_s, v1_s, v2_s, v3_s, v4_s, bcat_s, wg_s, wu_s, wd_s, cre_s, cim_s, cp_s,
            const_s, hc_s, col_s, coef_s, o_s, xn_s, sems):
    vecs = (v0_s, v1_s, v2_s, v3_s, v4_s)

    def cp(src, dst, k):
        return pltpu.make_async_copy(src, dst, sems.at[k])

    def wait_all(group):
        for c in group:
            c.wait()

    xw = M // 2
    g_vec = [cp(src, vecs[n], S_VEC)
             for n, src in enumerate((lre_hbm, lim_hbm, ldt_hbm, dsk_hbm, gw_hbm))]
    g_xa = [cp(xt_hbm.at[:, pl.ds(0, xw)], xt_s.at[0, pl.ds(0, D), pl.ds(0, xw)], S_XA)]
    g_xb = [cp(xt_hbm.at[:, pl.ds(xw, xw)], xt_s.at[0, pl.ds(0, D), pl.ds(xw, xw)], S_XB)]
    g_bt = [cp(bre_hbm.at[pl.ds(384, 64), :], bcat_s.at[pl.ds(768, 64), :], S_BT),
            cp(bim_hbm.at[pl.ds(384, 64), :], bcat_s.at[pl.ds(832, 64), :], S_BT)]
    g_b0 = [cp(bre_hbm.at[pl.ds(0, 256), :], bcat_s.at[pl.ds(0, 256), :], S_B0)]
    g_b1 = [cp(bre_hbm.at[pl.ds(256, 128), :], bcat_s.at[pl.ds(256, 128), :], S_B1)]
    g_b2 = [cp(bim_hbm.at[pl.ds(0, 384), :], bcat_s.at[pl.ds(384, 384), :], S_B2)]

    def w_cols(t0, t1, k):
        cols = pl.ds(t0 * FT, (t1 - t0) * FT)
        return [cp(src.at[:, cols], dst.at[pl.ds(0, D), cols], k)
                for src, dst in ((wg_hbm, wg_s), (wu_hbm, wu_s))]

    g_w0 = w_cols(0, T_W1, S_W0)
    g_w1 = w_cols(T_W1, T_W2, S_W1)
    g_wc = [cp(cre_hbm, cre_s.at[pl.ds(0, D), :], S_WC), cp(cim_hbm, cim_s, S_WC),
            cp(xt_hbm.at[:, pl.ds(M, M)], xt_s.at[1, pl.ds(0, D), :], S_WC)]
    g_w2 = w_cols(T_W2, NT, S_W2) + [cp(wdt_hbm, wd_s.at[pl.ds(0, D), :], S_W2)]
    g_w2 += [cp(xt_hbm.at[:, pl.ds(i * M, M)], xt_s.at[i, pl.ds(0, D), :], S_W2) for i in range(2, NC)]

    def pin(buf, row, piece):
        buf[row:row + PAD, 0:128] = piece.astype(BF16)

    def o_copy(i, s, r0, nr):
        return cp(o_s.at[i, pl.ds(r0, nr), pl.ds(s * 128, 128)],
                  o_hbm.at[pl.ds(r0, nr), pl.ds(i * M + s * 128, 128)], S_OUT)

    def start_all(group):
        for c in group:
            c.start()

    for group in (g_vec, g_xa, g_bt, g_xb):
        start_all(group)

    wait_all(g_vec)
    start_all(g_b0)

    def ext(v):
        return jnp.concatenate([v, v[:, 384:448]], axis=1)

    lre = vecs[0][...].astype(F32).reshape(1, D)
    lim = vecs[1][...].astype(F32).reshape(1, D)
    dt = jnp.exp(vecs[2][...].astype(F32).reshape(1, D)).astype(BF16).astype(F32)
    ar = dt * lre
    ai = dt * lim
    row = jax.lax.broadcasted_iota(jnp.int32, (8, 512), 0)
    lane = jax.lax.broadcasted_iota(jnp.int32, (8, 512), 1)
    k8 = (row + 1).astype(F32)
    mag = jnp.exp(k8 * ext(ar))
    ang = k8 * ext(ai)
    pr = mag * jnp.cos(ang)
    pi_ = mag * jnp.sin(ang) * jnp.where(lane >= D, -1.0, 1.0)
    const_s[0] = pr
    const_s[1] = pi_
    for n, kk in enumerate((1, 2, 4)):
        const_s[2 + 2 * n] = jnp.where(row >= kk, pr[kk - 1:kk, :], 0.0)
        const_s[3 + 2 * n] = jnp.where(row >= kk, pi_[kk - 1:kk, :], 0.0)
    hc_s[...] = jnp.zeros_like(hc_s)
    col_s[0] = jnp.broadcast_to(vecs[4][...].astype(F32).reshape(1, D), (128, D)).T
    col_s[1] = jnp.broadcast_to(vecs[3][...].astype(F32).reshape(1, D), (128, D)).T
    nre = pr[0:1, :D] - 1.0
    nim = pi_[0:1, :D]
    den = 1.0 / (lre * lre + lim * lim)
    coef_s[0] = jnp.broadcast_to(2.0 * ((nre * lre + nim * lim) * den), (8, D))
    coef_s[1] = jnp.broadcast_to(2.0 * ((nim * lre - nre * lim) * den), (8, D))

    def prep_c_block(r, cr8, ci8):
        rs = slice(r * 16, (r + 1) * 16)
        cr = jnp.concatenate([cr8, cr8], axis=0)
        ci = jnp.concatenate([ci8, ci8], axis=0)
        c_re = cre_s[rs, :].astype(F32)
        c_im = cim_s[rs, :].astype(F32)
        q_re = c_re * cr - c_im * ci
        q_im = -(c_re * ci + c_im * cr)
        cp_s[rs, 0:384] = q_re[:, 0:384].astype(BF16)
        cp_s[rs, 384:768] = q_im[:, 0:384].astype(BF16)
        cp_s[rs, 768:896] = jnp.concatenate(
            [q_re[:, 384:448], q_im[:, 384:448]], axis=1).astype(BF16)
        return (q_re[8:16, 0:128] + q_re[8:16, 128:256]) + (q_re[8:16, 256:384] + q_im[8:16, 256:384])

    def zero_after(v):
        return jnp.where(v < -jnp.inf, 1.0, 0.0)

    def chunk(i, first):
        if first:
            wait_all(g_xa)
            start_all(g_b1)
            xa = xt_s[0, 0:D, 0:xw].T
            pin(bcat_s, P2, xa[PIN_EARLY:PIN_EARLY + PAD, 0:128])
            wait_all(g_bt)
            start_all(g_b2)
            vta = _nt(xa, bcat_s[768:896, :])
            pin(xt_s.at[0], D, vta[2 * PIN_EARLY:2 * PIN_EARLY + PAD, :])
            wait_all(g_xb)
            start_all(g_w0)
            xb = xt_s[0, 0:D, xw:M].T
            vtb = _nt(xb, bcat_s[768:896, :])
            x = jnp.concatenate([xa, xb], axis=0)
        else:
            x = pltpu.bitcast(xn_s[...], BF16)
            g_first = jnp.dot(x, wg_s[0:D, 0:FT], preferred_element_type=F32)
        pr_ = slice(PIN_ROW, PIN_ROW + PAD)
        v_t = jnp.concatenate([vta, vtb], axis=0) if first else _nt(x, bcat_s[768:896, :])
        if first:
            pin(bcat_s, P2, vtb[PIN_ROW - 256:PIN_ROW - 256 + PAD, :])
            wait_all(g_b0)
            start_all(g_w1)
        v_r0 = _nt(x, bcat_s[0:256, :])
        if first:
            pin(bcat_s, P2, v_r0[pr_, 128:256])
            wait_all(g_b1)
            start_all(g_wc)
        v_r1 = _nt(x, bcat_s[256:384, :])
        if first:
            pin(bcat_s, P2, v_r1[pr_, :])
            wait_all(g_b2)
            start_all(g_w2)
        v_im = _nt(x, bcat_s[384:768, :])
        v_re = jnp.concatenate([v_r0, v_r1], axis=1)
        if first:
            pin(wg_s, D, v_im[pr_, 256:384])
            wait_all(g_w0)

        st = dict(c_re=hc_s[0], c_im=hc_s[1], g=0)
        hre, him = [], []

        def scan_group(z):
            gidx = st["g"]
            cs = [const_s[q] for q in range(8)]
            cs[2] = cs[2] + z
            cs[3] = cs[3] + z
            rs = slice(gidx * 8, gidx * 8 + 8)
            t = v_t[rs, :]
            vre = jnp.concatenate([v_re[rs, :], t], axis=1)
            vim = jnp.concatenate([v_im[rs, :], pltpu.roll(t, 64, 1)], axis=1)
            for n, kk in enumerate((1, 2, 4)):
                a_re, a_im = cs[2 + 2 * n], cs[3 + 2 * n]
                s_re = pltpu.roll(vre, kk, 0)
                s_im = pltpu.roll(vim, kk, 0)
                vre, vim = vre + (a_re * s_re - a_im * s_im), vim + (a_re * s_im + a_im * s_re)
            b_re = jnp.broadcast_to(st["c_re"][7:8, :], (8, 512))
            b_im = jnp.broadcast_to(st["c_im"][7:8, :], (8, 512))
            st["c_re"] = vre + (cs[0] * b_re - cs[1] * b_im)
            st["c_im"] = vim + (cs[0] * b_im + cs[1] * b_re)
            hre.append(st["c_re"])
            him.append(st["c_im"])
            st["g"] = gidx + 1

        hhs = []
        per = -(-NG // NT)
        npc = M // RB
        cblk = 0
        prev = None
        due = []
        for j in range(NT):
            if first and j == T_W1:
                pin(wg_s, D, prev)
                wait_all(g_w1)
            if first and j == T_WC:
                pin(cre_s, D, prev)
                wait_all(g_wc)
            if first and j == T_W2:
                pin(wd_s, D, prev)
                wait_all(g_w2)
            cols = slice(j * FT, (j + 1) * FT)
            g = g_first if j == 0 and not first else jnp.dot(
                x, wg_s[0:D, cols], preferred_element_type=F32)
            u = jnp.dot(x, wu_s[:, cols], preferred_element_type=F32)
            ng_here = min(per, NG - st["g"])
            g_trig = [(q * npc) // ng_here for q in range(ng_here)]
            c_trig = []
            if first and j >= T_PC:
                nblk = -(-(D // 16 - cblk) // (NT - j))
                c_trig = [((2 * q + 1) * npc) // (2 * nblk) for q in range(nblk)]
            c1 = GELU_C1
            if due:
                zs = [zero_after(v) for v in due]
                c1 = jnp.concatenate([GELU_C1 + sum(zs[1:], zs[0])] * (RB // 8), axis=0)
                due = []
            pieces = []
            for rb in range(npc):
                rs = slice(rb * RB, (rb + 1) * RB)
                gg = g[rs, :]
                inner = gg * (c1 + GELU_C2 * (gg * gg))
                r = gg * u[rs, :]
                pieces.append(r + r * jnp.tanh(inner))
                if rb in g_trig or rb in c_trig:
                    z = jnp.concatenate([zero_after(pieces[-1][0:8, :])] * 4, axis=1)
                    for _ in range(g_trig.count(rb)):
                        scan_group(z)
                    for _ in range(c_trig.count(rb)):
                        c_done = prep_c_block(cblk, coef_s[0] + z[:, :D], coef_s[1] + z[:, :D])
                        cblk += 1
            hhs.append(jnp.concatenate(pieces, axis=0))
            prev = pieces[PIN_PIECE][0:PAD, :]
            if first and ng_here:
                c = st["c_re"]
                due.append((c[:, 0:128] + c[:, 128:256]) + (c[:, 256:384] + c[:, 384:512]))
            if c_trig:
                due.append(c_done)
            if T_PF <= j < T_PF + NS:
                q = j - T_PF
                xq = xt_s[jnp.minimum(i + 1, NC - 1), 0:D, q * 128:(q + 1) * 128].T
                xn_s[q * 64:(q + 1) * 64, :] = pltpu.bitcast(xq, jnp.uint32)
                if first:
                    xf = xq[112:128, :].astype(F32)[8:16, :]
                    due.append((xf[:, 0:128] + xf[:, 128:256]) + (
                        xf[:, 256:384] + jnp.concatenate([xf[:, 384:448]] * 2, axis=1)))
        assert st["g"] == NG and cblk == (D // 16 if first else 0)
        hc_s[0] = st["c_re"]
        hc_s[1] = st["c_im"]
        h_re = jnp.concatenate(hre, axis=0)
        h_im = jnp.concatenate(him, axis=0)
        hp = jnp.concatenate([h_re[:, :384], h_im[:, :384], h_re[:, 384:]], axis=1)
        hh = jnp.concatenate(hhs, axis=1)

        for s in range(NS):
            sl = slice(s * 128, (s + 1) * 128)
            xtf = xt_s[i, 0:D, sl].astype(F32)
            a = _nt(cp_s[...], hp[sl, :].astype(BF16)) + xtf * col_s[1]
            b = _nt(wd_s[0:D, :], hh[sl, :].astype(BF16))
            gate = jax.nn.sigmoid(jnp.sum(xtf * col_s[0], axis=0, keepdims=True))
            g1 = 0.5 * (1.0 - gate)
            nsp = OSPLIT if s == NS - 1 else 1
            nr = D // nsp
            for q in range(nsp):
                rr = slice(q * nr, (q + 1) * nr)
                o_s[i, rr, sl] = gate * a[rr, :] + g1 * b[rr, :]
                o_copy(i, s, q * nr, nr).start()

    chunk(0, True)

    def body(i, carry):
        chunk(i, False)
        return carry

    jax.lax.fori_loop(1, NC, body, 0)
    pltpu.make_async_copy(o_s, o_s, sems.at[S_OUT]).wait()


@jax.jit
def pallas_gated_mix__ssm_conv_s5__glu_gated_geglu__prompt_kernel(
    A_x: jax.Array,
    A_Lambda_re: jax.Array,
    A_Lambda_im: jax.Array,
    A_B_re: jax.Array,
    A_B_im: jax.Array,
    A_C_re: jax.Array,
    A_C_im: jax.Array,
    A_log_dt: jax.Array,
    A_Dskip: jax.Array,
    B_x: jax.Array,
    B_w_gate: jax.Array,
    B_w_up: jax.Array,
    B_w_down: jax.Array,
    gate_w: jax.Array,
):
    del B_x
    assert A_x.shape == (1, S, D) and B_w_gate.shape == (D, F) and B_w_down.shape == (F, D)
    xt = jnp.transpose(A_x.reshape(S, D))
    wdt = jnp.transpose(B_w_down)
    hbm = pl.BlockSpec(memory_space=pl.ANY)
    out_t = pl.pallas_call(
        _kernel,
        in_specs=[hbm] * 13,
        out_specs=hbm,
        out_shape=jax.ShapeDtypeStruct((D, S), F32),
        scratch_shapes=[
            pltpu.VMEM((NC, D + PAD, M), BF16),
            pltpu.VMEM((D,), BF16), pltpu.VMEM((D,), BF16), pltpu.VMEM((D,), BF16),
            pltpu.VMEM((D,), BF16), pltpu.VMEM((D,), BF16),
            pltpu.VMEM((P2 + PAD, D), BF16),
            pltpu.VMEM((D + PAD, F), BF16),
            pltpu.VMEM((D, F), BF16),
            pltpu.VMEM((D + PAD, F), BF16),
            pltpu.VMEM((D + PAD, D), BF16),
            pltpu.VMEM((D, D), BF16),
            pltpu.VMEM((D, P2), BF16),
            pltpu.VMEM((8, 8, 512), F32),
            pltpu.VMEM((2, 8, 512), F32),
            pltpu.VMEM((2, D, 128), F32),
            pltpu.VMEM((2, 8, D), F32),
            pltpu.VMEM((NC, D, M), F32),
            pltpu.VMEM((M // 2, D), jnp.uint32),
            pltpu.SemaphoreType.DMA((N_SEMS,)),
        ],
        compiler_params=pltpu.CompilerParams(
            vmem_limit_bytes=100 * 1024 * 1024,
            flags={"XLA_TPU_RESCHEDULE_DMA_DONES": True}),
    )(xt, A_Lambda_re, A_Lambda_im, A_B_re, A_B_im, A_C_re, A_C_im, A_log_dt, A_Dskip,
      B_w_gate, B_w_up, wdt, gate_w)
    return jnp.transpose(out_t).reshape(1, S, D)
```

```python
import jax
import jax.numpy as jnp
import jax.experimental.pallas as pl
import jax.experimental.pallas.tpu as pltpu

F32 = jnp.float32
BF16 = jnp.bfloat16

S = 2048
D = 448
F = 1792
P2 = 2 * D
M = 512
NC = S // M
NS = M // 128
NG = M // 8
FT = 128
NT = F // FT
RB = 32
T_W1 = 4
T_WC = 8
T_W2 = 12
T_PC = 9
T_PF = 9
PIN_EARLY = 48
PIN_ROW = 288
PIN_PIECE = 8
PAD = 16
GELU_C1 = 0.7978845608028654
GELU_C2 = 0.7978845608028654 * 0.044715

S_VEC = S_B0 = S_W1 = 0
S_XA = S_B1 = S_WC = 1
S_XB = S_W0 = 2
S_BT = S_B2 = S_W2 = 3
N_SEMS = 4
assert NS <= N_SEMS

_FLAGS = ({"XLA_TPU_RESCHEDULE_DMA_DONES": True} if jax.__version__.startswith("0.12.") else {})


def _nt(a, b):
    return jax.lax.dot_general(a, b, (((1,), (1,)), ((), ())), preferred_element_type=F32)


def _kernel(xt_hbm, lre_hbm, lim_hbm, bre_hbm, bim_hbm, cre_hbm, cim_hbm, ldt_hbm, dsk_hbm,
            wg_hbm, wu_hbm, wdt_hbm, gw_hbm, o_hbm,
            xt_s, v0_s, v1_s, v2_s, v3_s, v4_s, bcat_s, wg_s, wu_s, wd_s, cre_s, cim_s, cp_s,
            const_s, hc_s, col_s, coef_s, o_s, xn_s, sems):
    vecs = (v0_s, v1_s, v2_s, v3_s, v4_s)

    def cp(src, dst, k):
        return pltpu.make_async_copy(src, dst, sems.at[k])

    def wait_all(group):
        for c in group:
            c.wait()

    xw = M // 2
    g_vec = [cp(src, vecs[n], S_VEC)
             for n, src in enumerate((lre_hbm, lim_hbm, ldt_hbm, dsk_hbm, gw_hbm))]
    g_xa = [cp(xt_hbm.at[:, pl.ds(0, xw)], xt_s.at[0, pl.ds(0, D), pl.ds(0, xw)], S_XA)]
    g_xb = [cp(xt_hbm.at[:, pl.ds(xw, xw)], xt_s.at[0, pl.ds(0, D), pl.ds(xw, xw)], S_XB)]
    g_bt = [cp(bre_hbm.at[pl.ds(384, 64), :], bcat_s.at[pl.ds(768, 64), :], S_BT),
            cp(bim_hbm.at[pl.ds(384, 64), :], bcat_s.at[pl.ds(832, 64), :], S_BT)]
    g_b0 = [cp(bre_hbm.at[pl.ds(0, 256), :], bcat_s.at[pl.ds(0, 256), :], S_B0)]
    g_b1 = [cp(bre_hbm.at[pl.ds(256, 128), :], bcat_s.at[pl.ds(256, 128), :], S_B1)]
    g_b2 = [cp(bim_hbm.at[pl.ds(0, 384), :], bcat_s.at[pl.ds(384, 384), :], S_B2)]

    def w_cols(t0, t1, k):
        cols = pl.ds(t0 * FT, (t1 - t0) * FT)
        return [cp(src.at[:, cols], dst.at[pl.ds(0, D), cols], k)
                for src, dst in ((wg_hbm, wg_s), (wu_hbm, wu_s))]

    g_w0 = w_cols(0, T_W1, S_W0)
    g_w1 = w_cols(T_W1, T_W2, S_W1)
    g_wc = [cp(cre_hbm, cre_s.at[pl.ds(0, D), :], S_WC), cp(cim_hbm, cim_s, S_WC),
            cp(xt_hbm.at[:, pl.ds(M, M)], xt_s.at[1, pl.ds(0, D), :], S_WC)]
    g_w2 = w_cols(T_W2, NT, S_W2) + [cp(wdt_hbm, wd_s.at[pl.ds(0, D), :], S_W2)]
    g_w2 += [cp(xt_hbm.at[:, pl.ds(i * M, M)], xt_s.at[i, pl.ds(0, D), :], S_W2) for i in range(2, NC)]

    def pin(buf, row, piece):
        buf[row:row + PAD, 0:128] = piece.astype(BF16)

    def o_copy(i, s):
        return cp(o_s.at[i, :, pl.ds(s * 128, 128)], o_hbm.at[:, pl.ds(i * M + s * 128, 128)], s)

    def start_all(group):
        for c in group:
            c.start()

    for group in (g_vec, g_xa, g_bt, g_xb):
        start_all(group)

    wait_all(g_vec)
    start_all(g_b0)

    def ext(v):
        return jnp.concatenate([v, v[:, 384:448]], axis=1)

    lre = vecs[0][...].astype(F32).reshape(1, D)
    lim = vecs[1][...].astype(F32).reshape(1, D)
    dt = jnp.exp(vecs[2][...].astype(F32).reshape(1, D)).astype(BF16).astype(F32)
    ar = dt * lre
    ai = dt * lim
    row = jax.lax.broadcasted_iota(jnp.int32, (8, 512), 0)
    lane = jax.lax.broadcasted_iota(jnp.int32, (8, 512), 1)
    k8 = (row + 1).astype(F32)
    mag = jnp.exp(k8 * ext(ar))
    ang = k8 * ext(ai)
    pr = mag * jnp.cos(ang)
    pi_ = mag * jnp.sin(ang) * jnp.where(lane >= D, -1.0, 1.0)
    const_s[0] = pr
    const_s[1] = pi_
    for n, kk in enumerate((1, 2, 4)):
        const_s[2 + 2 * n] = jnp.where(row >= kk, pr[kk - 1:kk, :], 0.0)
        const_s[3 + 2 * n] = jnp.where(row >= kk, pi_[kk - 1:kk, :], 0.0)
    hc_s[...] = jnp.zeros_like(hc_s)
    col_s[0] = jnp.broadcast_to(vecs[4][...].astype(F32).reshape(1, D), (128, D)).T
    col_s[1] = jnp.broadcast_to(vecs[3][...].astype(F32).reshape(1, D), (128, D)).T
    nre = pr[0:1, :D] - 1.0
    nim = pi_[0:1, :D]
    den = 1.0 / (lre * lre + lim * lim)
    coef_s[0] = jnp.broadcast_to(2.0 * ((nre * lre + nim * lim) * den), (8, D))
    coef_s[1] = jnp.broadcast_to(2.0 * ((nim * lre - nre * lim) * den), (8, D))

    def prep_c_block(r, cr8, ci8):
        rs = slice(r * 16, (r + 1) * 16)
        cr = jnp.concatenate([cr8, cr8], axis=0)
        ci = jnp.concatenate([ci8, ci8], axis=0)
        c_re = cre_s[rs, :].astype(F32)
        c_im = cim_s[rs, :].astype(F32)
        q_re = c_re * cr - c_im * ci
        q_im = -(c_re * ci + c_im * cr)
        cp_s[rs, 0:384] = q_re[:, 0:384].astype(BF16)
        cp_s[rs, 384:768] = q_im[:, 0:384].astype(BF16)
        cp_s[rs, 768:896] = jnp.concatenate(
            [q_re[:, 384:448], q_im[:, 384:448]], axis=1).astype(BF16)
        return (q_re[8:16, 0:128] + q_re[8:16, 128:256]) + (q_re[8:16, 256:384] + q_im[8:16, 256:384])

    def zero_after(v):
        return jnp.where(v < -jnp.inf, 1.0, 0.0)

    def chunk(i, first):
        if first:
            wait_all(g_xa)
            start_all(g_b1)
            xa = xt_s[0, 0:D, 0:xw].T
            pin(bcat_s, P2, xa[PIN_EARLY:PIN_EARLY + PAD, 0:128])
            wait_all(g_bt)
            start_all(g_b2)
            vta = _nt(xa, bcat_s[768:896, :])
            pin(xt_s.at[0], D, vta[2 * PIN_EARLY:2 * PIN_EARLY + PAD, :])
            wait_all(g_xb)
            start_all(g_w0)
            xb = xt_s[0, 0:D, xw:M].T
            vtb = _nt(xb, bcat_s[768:896, :])
            x = jnp.concatenate([xa, xb], axis=0)
        else:
            x = pltpu.bitcast(xn_s[...], BF16)
            g_first = jnp.dot(x, wg_s[0:D, 0:FT], preferred_element_type=F32)
        pr_ = slice(PIN_ROW, PIN_ROW + PAD)
        v_t = jnp.concatenate([vta, vtb], axis=0) if first else _nt(x, bcat_s[768:896, :])
        if first:
            pin(bcat_s, P2, v_t[pr_, :])
            wait_all(g_b0)
            start_all(g_w1)
        v_r0 = _nt(x, bcat_s[0:256, :])
        if first:
            pin(bcat_s, P2, v_r0[pr_, 128:256])
            wait_all(g_b1)
            start_all(g_wc)
        v_r1 = _nt(x, bcat_s[256:384, :])
        if first:
            pin(bcat_s, P2, v_r1[pr_, :])
            wait_all(g_b2)
            start_all(g_w2)
        v_im = _nt(x, bcat_s[384:768, :])
        v_re = jnp.concatenate([v_r0, v_r1], axis=1)
        if first:
            pin(wg_s, D, v_im[pr_, 256:384])
            wait_all(g_w0)

        st = dict(c_re=hc_s[0], c_im=hc_s[1], g=0)
        hre, him = [], []

        def scan_group(z):
            gidx = st["g"]
            cs = [const_s[q] for q in range(8)]
            cs[2] = cs[2] + z
            cs[3] = cs[3] + z
            rs = slice(gidx * 8, gidx * 8 + 8)
            t = v_t[rs, :]
            vre = jnp.concatenate([v_re[rs, :], t], axis=1)
            vim = jnp.concatenate([v_im[rs, :], pltpu.roll(t, 64, 1)], axis=1)
            for n, kk in enumerate((1, 2, 4)):
                a_re, a_im = cs[2 + 2 * n], cs[3 + 2 * n]
                s_re = pltpu.roll(vre, kk, 0)
                s_im = pltpu.roll(vim, kk, 0)
                vre, vim = vre + (a_re * s_re - a_im * s_im), vim + (a_re * s_im + a_im * s_re)
            b_re = jnp.broadcast_to(st["c_re"][7:8, :], (8, 512))
            b_im = jnp.broadcast_to(st["c_im"][7:8, :], (8, 512))
            st["c_re"] = vre + (cs[0] * b_re - cs[1] * b_im)
            st["c_im"] = vim + (cs[0] * b_im + cs[1] * b_re)
            hre.append(st["c_re"])
            him.append(st["c_im"])
            st["g"] = gidx + 1

        hhs = []
        per = -(-NG // NT)
        npc = M // RB
        cblk = 0
        prev = None
        due = []
        for j in range(NT):
            if first and j == T_W1:
                pin(wg_s, D, prev)
                wait_all(g_w1)
            if first and j == T_WC:
                pin(cre_s, D, prev)
                wait_all(g_wc)
            if first and j == T_W2:
                pin(wd_s, D, prev)
                wait_all(g_w2)
            cols = slice(j * FT, (j + 1) * FT)
            g = g_first if j == 0 and not first else jnp.dot(
                x, wg_s[0:D, cols], preferred_element_type=F32)
            u = jnp.dot(x, wu_s[:, cols], preferred_element_type=F32)
            ng_here = min(per, NG - st["g"])
            g_trig = [(q * npc) // ng_here for q in range(ng_here)]
            c_trig = []
            if first and j >= T_PC:
                nblk = -(-(D // 16 - cblk) // (NT - j))
                c_trig = [((2 * q + 1) * npc) // (2 * nblk) for q in range(nblk)]
            c1 = GELU_C1
            if due:
                zs = [zero_after(v) for v in due]
                c1 = jnp.concatenate([GELU_C1 + sum(zs[1:], zs[0])] * (RB // 8), axis=0)
                due = []
            pieces = []
            for rb in range(npc):
                rs = slice(rb * RB, (rb + 1) * RB)
                gg = g[rs, :]
                inner = gg * (c1 + GELU_C2 * (gg * gg))
                r = gg * u[rs, :]
                pieces.append(r + r * jnp.tanh(inner))
                if rb in g_trig or rb in c_trig:
                    z = jnp.concatenate([zero_after(pieces[-1][0:8, :])] * 4, axis=1)
                    for _ in range(g_trig.count(rb)):
                        scan_group(z)
                    for _ in range(c_trig.count(rb)):
                        c_done = prep_c_block(cblk, coef_s[0] + z[:, :D], coef_s[1] + z[:, :D])
                        cblk += 1
            hhs.append(jnp.concatenate(pieces, axis=0))
            prev = pieces[PIN_PIECE][0:PAD, :]
            if first and ng_here:
                c = st["c_re"]
                due.append((c[:, 0:128] + c[:, 128:256]) + (c[:, 256:384] + c[:, 384:512]))
            if c_trig:
                due.append(c_done)
            if T_PF <= j < T_PF + NS:
                q = j - T_PF
                xq = xt_s[jnp.minimum(i + 1, NC - 1), 0:D, q * 128:(q + 1) * 128].T
                xn_s[q * 64:(q + 1) * 64, :] = pltpu.bitcast(xq, jnp.uint32)
                if first:
                    xf = xq[112:128, :].astype(F32)[8:16, :]
                    due.append((xf[:, 0:128] + xf[:, 128:256]) + (
                        xf[:, 256:384] + jnp.concatenate([xf[:, 384:448]] * 2, axis=1)))
        assert st["g"] == NG and cblk == (D // 16 if first else 0)
        hc_s[0] = st["c_re"]
        hc_s[1] = st["c_im"]
        h_re = jnp.concatenate(hre, axis=0)
        h_im = jnp.concatenate(him, axis=0)
        hp = jnp.concatenate([h_re[:, :384], h_im[:, :384], h_re[:, 384:]], axis=1)
        hh = jnp.concatenate(hhs, axis=1)

        if not first:
            o_s[jnp.minimum(i + 1, NC - 1), 0:8, 0:128] = prev[0:8, :]
            wait_all([o_copy(i - 1, s) for s in range(NS)])

        for s in range(NS):
            sl = slice(s * 128, (s + 1) * 128)
            xtf = xt_s[i, 0:D, sl].astype(F32)
            a = _nt(cp_s[...], hp[sl, :].astype(BF16)) + xtf * col_s[1]
            b = _nt(wd_s[0:D, :], hh[sl, :].astype(BF16))
            gate = jax.nn.sigmoid(jnp.sum(xtf * col_s[0], axis=0, keepdims=True))
            g1 = 0.5 * (1.0 - gate)
            o_s[i, :, sl] = gate * a + g1 * b
            o_copy(i, s).start()

    chunk(0, True)

    def body(i, carry):
        chunk(i, False)
        return carry

    jax.lax.fori_loop(1, NC, body, 0)
    wait_all([o_copy(NC - 1, s) for s in range(NS)])


@jax.jit
def pallas_gated_mix__ssm_conv_s5__glu_gated_geglu__prompt_kernel(
    A_x: jax.Array,
    A_Lambda_re: jax.Array,
    A_Lambda_im: jax.Array,
    A_B_re: jax.Array,
    A_B_im: jax.Array,
    A_C_re: jax.Array,
    A_C_im: jax.Array,
    A_log_dt: jax.Array,
    A_Dskip: jax.Array,
    B_x: jax.Array,
    B_w_gate: jax.Array,
    B_w_up: jax.Array,
    B_w_down: jax.Array,
    gate_w: jax.Array,
):
    del B_x
    assert A_x.shape == (1, S, D) and B_w_gate.shape == (D, F) and B_w_down.shape == (F, D)
    xt = jnp.transpose(A_x.reshape(S, D))
    wdt = jnp.transpose(B_w_down)
    hbm = pl.BlockSpec(memory_space=pl.ANY)
    out_t = pl.pallas_call(
        _kernel,
        in_specs=[hbm] * 13,
        out_specs=hbm,
        out_shape=jax.ShapeDtypeStruct((D, S), F32),
        scratch_shapes=[
            pltpu.VMEM((NC, D + PAD, M), BF16),
            pltpu.VMEM((D,), BF16), pltpu.VMEM((D,), BF16), pltpu.VMEM((D,), BF16),
            pltpu.VMEM((D,), BF16), pltpu.VMEM((D,), BF16),
            pltpu.VMEM((P2 + PAD, D), BF16),
            pltpu.VMEM((D + PAD, F), BF16),
            pltpu.VMEM((D, F), BF16),
            pltpu.VMEM((D + PAD, F), BF16),
            pltpu.VMEM((D + PAD, D), BF16),
            pltpu.VMEM((D, D), BF16),
            pltpu.VMEM((D, P2), BF16),
            pltpu.VMEM((8, 8, 512), F32),
            pltpu.VMEM((2, 8, 512), F32),
            pltpu.VMEM((2, D, 128), F32),
            pltpu.VMEM((2, 8, D), F32),
            pltpu.VMEM((NC, D, M), F32),
            pltpu.VMEM((M // 2, D), jnp.uint32),
            pltpu.SemaphoreType.DMA((N_SEMS,)),
        ],
        compiler_params=pltpu.CompilerParams(
            vmem_limit_bytes=100 * 1024 * 1024, flags=_FLAGS),
    )(xt, A_Lambda_re, A_Lambda_im, A_B_re, A_B_im, A_C_re, A_C_im, A_log_dt, A_Dskip,
      B_w_gate, B_w_up, wdt, gate_w)
    return jnp.transpose(out_t).reshape(1, S, D)
```
